```python
import jax
import jax.numpy as jnp

def _softmax(x, axis=-1):
    return jax.nn.softmax(x, axis=axis)
def _gelu(x):
    return jax.nn.gelu(x, approximate=True)
def _silu(x):
    return jax.nn.silu(x)
def _sigmoid(x):
    return jax.nn.sigmoid(x)
def _layernorm(x, axis=-1, eps=1e-5):
    m = jnp.mean(x, axis=axis, keepdims=True)
    v = jnp.var(x, axis=axis, keepdims=True)
    return (x - m) / jnp.sqrt(v + eps)
def _scatter_add(tgt, idx, src, axis=0):
    return tgt.at[idx].add(src)
def _segment_sum(src, seg, n):
    return jax.ops.segment_sum(src, seg, n)
class _Rng:
    def __init__(self, key):
        self._k = key
    def _next(self):
        self._k, sub = jax.random.split(self._k)
        return sub
    def normal(self, shape):
        return jax.random.normal(self._next(), shape, dtype=jnp.bfloat16)
    def randint(self, lo, hi, shape):
        return jax.random.randint(self._next(), shape, lo, hi, dtype=jnp.int32)
    def uniform(self, shape, lo=0.0, hi=1.0):
        return jax.random.uniform(self._next(), shape, jnp.bfloat16, lo, hi)
    def permutation(self, n):
        return jax.random.permutation(self._next(), n)


kernel_name = 'standalone__modern_conv_block_slak__vision'

def setup_inputs():
    _rng = _Rng(jax.random.key(int.from_bytes(__import__("os").urandom(4), "little")))
    _w = (lambda a: (lambda t: t.astype(jnp.bfloat16) if jnp.issubdtype(t.dtype, jnp.floating) else t)(jnp.asarray(a)))
    H = W = 384
    C = 384
    K = 1
    return {
        "x": _w((lambda *s: _rng.normal(s) * 0.05)(1, H, W, C)),
        "dw": _w((lambda *s: _rng.normal(s) * 0.05)(K, K, C)),
        "w1": _w((lambda *s: _rng.normal(s) * 0.05)(C, 4 * C)),
        "w2": _w((lambda *s: _rng.normal(s) * 0.05)(4 * C, C)),
        "grn_g": _w((lambda *s: _rng.normal(s) * 0.05)(4 * C)),
        "grn_b": _w((lambda *s: _rng.normal(s) * 0.05)(4 * C)),
    }

def reference(x, dw, w1, w2, grn_g, grn_b):
    B, H, W, C = x.shape
    K = dw.shape[0]
    pad = K // 2
    xp = jnp.pad(x, ((0,0),(pad,pad),(pad,pad),(0,0)))
    out = jnp.zeros_like(x)
    for i in range(K):
        for j in range(K):
            out = out + xp[:, i:i+H, j:j+W, :] * dw[i, j][None, None, None, :]
    h = _layernorm(out, axis=-1)
    h = _gelu(h @ w1)
    gx = jnp.sqrt((h * h).sum(axis=(1, 2), keepdims=True) + 1e-6)
    nx = gx / (gx.mean(axis=-1, keepdims=True) + 1e-6)
    h = grn_g[None, None, None, :] * (h * nx) + grn_b[None, None, None, :] + h
    return x + h @ w2
```

```python
import functools
import math

import jax
import jax.numpy as jnp
import jax.experimental.pallas as pl
import jax.experimental.pallas.tpu as pltpu

F32 = jnp.float32
BF16 = jnp.bfloat16
U32 = jnp.uint32

LN_EPS = 1e-5
GRN_EPS = 1e-6
_C0 = 0.7978845608028654
_C1 = 0.044715
ALPHA = (_C0 * _C1) ** (1.0 / 3.0)
A0 = _C0 / ALPHA
KH = 0.5 / ALPHA


def _split_rows(total, parts, align=16):
    units = total // align
    base, rem = divmod(units, parts)
    sizes = [(base + (1 if k < rem else 0)) * align for k in range(parts)]
    offs = [sum(sizes[:k]) for k in range(parts)]
    return list(zip(offs, sizes))


def _kernel(x_hbm, dw_ref, w1_hbm, w2_hbm, g_ref, b_ref,
            out_hbm, h_hbm,
            hpool, nbuf, xbuf, obuf, w1v, w2v, w2s, ssq, bias,
            hsem, xsem, osem, psem, wsem,
            *, T, S, tm, sub, nc, sub2, margin):
    C = x_hbm.shape[1]
    N = w1_hbm.shape[1]
    NH = T - S
    U = tm // sub
    U2 = tm // sub2

    def h_wr(tile, slot):
        return pltpu.make_async_copy(
            hpool.at[slot], h_hbm.at[pl.ds(tile * tm, tm), :], hsem.at[slot])

    def h_rd(tile, slot):
        return pltpu.make_async_copy(
            h_hbm.at[pl.ds(tile * tm, tm), :], hpool.at[slot], hsem.at[slot])

    def x_cp(tile, b):
        return pltpu.make_async_copy(
            x_hbm.at[pl.ds(tile * tm, tm), :], xbuf.at[b], xsem.at[b])

    def x0_cp(j):
        return pltpu.make_async_copy(
            x_hbm.at[pl.ds(j * sub, sub), :], xbuf.at[0, pl.ds(j * sub, sub), :], psem.at[j])

    def o_part(tile, b, j):
        return pltpu.make_async_copy(
            obuf.at[b, pl.ds(j * sub2, sub2), :],
            out_hbm.at[pl.ds(tile * tm + j * sub2, sub2), :], osem.at[b])

    def o_all(tile, b):
        return pltpu.make_async_copy(
            obuf.at[b], out_hbm.at[pl.ds(tile * tm, tm), :], osem.at[b])

    w1_cp = pltpu.make_async_copy(w1_hbm, w1v, wsem.at[0])
    w2_cp = pltpu.make_async_copy(w2_hbm, w2v, wsem.at[1])

    def wrap(v, n):
        return jnp.where(v >= n, v - n, v)

    def ln_piece(xb, dst, r0, rows):
        dw = dw_ref[...].astype(F32)
        y = xbuf[xb, r0:r0 + rows, :].astype(F32) * dw
        m = jnp.sum(y, axis=-1, keepdims=True) * (1.0 / C)
        d = y - m
        ss = jnp.sum(d * d, axis=-1, keepdims=True)
        r = jnp.exp(jnp.log(ss + C * LN_EPS) * (-0.5) + math.log(ALPHA * C ** 0.5))
        n = (d * r).astype(BF16)
        nbuf[dst, r0 // 2:(r0 + rows) // 2, :] = pltpu.bitcast(n, U32)

    def mm1(cur, slot, j, c, order):
        r0 = j * sub
        parts = [pltpu.bitcast(nbuf[cur, (r0 + o) // 2:(r0 + o + r) // 2, :], BF16)
                 for (o, r) in order]
        lhs = parts[0] if len(parts) == 1 else jnp.concatenate(parts, axis=0)
        u = jnp.dot(lhs, w1v[:, c * nc:(c + 1) * nc], preferred_element_type=F32)
        h = u + u * jnp.tanh(u * (u * u + A0))
        pos = 0
        for (o, r) in order:
            hpool[slot, r0 + o:r0 + o + r, c * nc:(c + 1) * nc] = h[pos:pos + r, :].astype(BF16)
            pos += r
        ssq[:, c * nc:(c + 1) * nc] += (h * h).reshape(sub // 8, 8, nc).sum(axis=0)

    def x_seq(m):
        return jnp.where(m < T, m, wrap(m - T + NH, T))

    for j in range(U):
        x0_cp(j).start()
    w1_cp.start()
    x_cp(1, 1).start()
    w2_cp.start()
    ssq[...] = jnp.zeros_like(ssq)
    for j in range(U):
        x0_cp(j).wait()
        for (o, r) in _split_rows(sub, max(sub // 256, 1)):
            ln_piece(0, 0, j * sub + o, r)
    x_cp(2, 0).start()
    w1_cp.wait()

    def phase0(i, slot):
        cur = i & 1
        nxt = 1 - cur
        x_cp(x_seq(i + 1), nxt).wait()

        @pl.when(i >= S)
        def _():
            h_wr(i - S, slot).wait()

        nch = N // nc
        sp = _split_rows(sub, nch)
        pieces = [(j * sub + o, r) for j in range(U) for (o, r) in sp]
        P = len(pieces)
        for j in range(U):
            for c in range(nch):
                order = [sp[k] for k in range(nch) if k != c] + [sp[c]]
                q = j * nch + c
                mm1(cur, slot, j, c, order)
                if q == P - 2:
                    ln_piece(nxt, nxt, *pieces[P - 1])
                    ln_piece(nxt, nxt, *pieces[0])
                elif q < P - 2:
                    ln_piece(nxt, nxt, *pieces[q + 1])

        @pl.when(i + 3 <= T + 1)
        def _():
            x_cp(x_seq(i + 3), nxt).start()

        @pl.when(i < NH)
        def _():
            h_wr(i, slot).start()

        return wrap(slot + 1, S)

    jax.lax.fori_loop(0, T, phase0, 0)

    w2_cp.wait()
    tot = jnp.sum(ssq[...], axis=0, keepdims=True) * (KH * KH)
    gx = jnp.sqrt(tot + GRN_EPS)
    nx = gx / (jnp.mean(gx, axis=-1, keepdims=True) + GRN_EPS)
    s = (1.0 + g_ref[...].astype(F32) * nx) * KH
    st = jnp.transpose(jnp.broadcast_to(s, (128, N)))
    w2 = w2v[...]
    w2f = w2.astype(F32)
    for c in range(C // 128):
        w2s[:, c * 128:(c + 1) * 128] = (w2f[:, c * 128:(c + 1) * 128] * st).astype(BF16)
    bias[...] = jnp.dot(jnp.broadcast_to(b_ref[...], (16, N)), w2,
                        preferred_element_type=F32)[:8]

    num, den = (S - margin) + (NH - 1), (NH - 1)

    def phase1(i, carry):
        slot, tile, tile2, kk, kslot, acc = carry
        xb = (T + i) & 1
        ob = i & 1

        @pl.when(i >= 1)
        def _():
            x_cp(tile, xb).wait()

        @pl.when(i >= S)
        def _():
            h_rd(i - S, slot).wait()

        @pl.when(i >= 2)
        def _():
            o_all(tile2, ob).wait()

        bi = bias[0:1, :]
        for j in range(U2):
            r0 = j * sub2
            y = jnp.dot(hpool[slot, r0:r0 + sub2, :], w2s[...], preferred_element_type=F32)
            obuf[ob, r0:r0 + sub2, :] = (
                xbuf[xb, r0:r0 + sub2, :].astype(F32) + y + bi).astype(BF16)
            o_part(tile, ob, j).start()

        @pl.when(i + 2 < T)
        def _():
            x_cp(wrap(tile + 2, T), xb).start()

        hit = jnp.logical_and(acc < den, kk < NH)

        @pl.when(hit)
        def _():
            h_rd(kk, kslot).start(priority=1)

        acc = jnp.where(hit, acc + num, acc) - den
        kk = jnp.where(hit, kk + 1, kk)
        kslot = jnp.where(hit, wrap(kslot + 1, S), kslot)
        tile2 = wrap(tile + (T - 1), T)
        return wrap(slot + 1, S), wrap(tile + 1, T), tile2, kk, kslot, acc

    zero = jnp.int32(0)
    jax.lax.fori_loop(0, T, phase1,
                      (jnp.int32(NH % S), jnp.int32(NH % T), zero, zero, jnp.int32(NH % S), zero))
    o_all((NH + T - 2) % T, (T - 2) % 2).wait()
    o_all((NH + T - 1) % T, (T - 1) % 2).wait()


def _build(tm=3072, S=11, sub=512, nc=256, sub2=512, margin=3, vmem_mb=124):
    def fn(x, dw, w1, w2, grn_g, grn_b):
        B, H, W, C = x.shape
        M = B * H * W
        N = w1.shape[1]
        T = M // tm
        NH = T - S
        assert dw.shape[0] == 1 and dw.shape[1] == 1 and B == 1
        assert M % tm == 0 and NH >= 2 and T >= 3
        vm = pl.BlockSpec(memory_space=pltpu.VMEM)
        hbm = pl.BlockSpec(memory_space=pl.ANY)
        out, _ = pl.pallas_call(
            functools.partial(_kernel, T=T, S=S, tm=tm, sub=sub, nc=nc, sub2=sub2,
                              margin=margin),
            in_specs=[hbm, vm, hbm, hbm, vm, vm],
            out_specs=[hbm, hbm],
            out_shape=[
                jax.ShapeDtypeStruct((M, C), BF16),
                jax.ShapeDtypeStruct((NH * tm, N), BF16),
            ],
            scratch_shapes=[
                pltpu.VMEM((S, tm, N), BF16),
                pltpu.VMEM((2, tm // 2, C), U32),
                pltpu.VMEM((2, tm, C), BF16),
                pltpu.VMEM((2, tm, C), BF16),
                pltpu.VMEM((C, N), BF16),
                pltpu.VMEM((N, C), BF16),
                pltpu.VMEM((N, C), BF16),
                pltpu.VMEM((8, N), F32),
                pltpu.VMEM((8, C), F32),
                pltpu.SemaphoreType.DMA((S,)),
                pltpu.SemaphoreType.DMA((2,)),
                pltpu.SemaphoreType.DMA((2,)),
                pltpu.SemaphoreType.DMA((tm // sub,)),
                pltpu.SemaphoreType.DMA((2,)),
            ],
            compiler_params=pltpu.CompilerParams(
                vmem_limit_bytes=vmem_mb * 1024 * 1024,
                disable_bounds_checks=True,
            ),
        )(x.reshape(M, C), dw.reshape(1, C), w1, w2,
          grn_g.reshape(1, N), grn_b.reshape(1, N))
        return out.reshape(B, H, W, C)

    return fn


_impl = _build()


@jax.jit
def pallas_standalone__modern_conv_block_slak__vision_kernel(
    x: jax.Array,
    dw: jax.Array,
    w1: jax.Array,
    w2: jax.Array,
    grn_g: jax.Array,
    grn_b: jax.Array,
):
    return _impl(x, dw, w1, w2, grn_g, grn_b)
```

```python
import functools
import math

import jax
import jax.numpy as jnp
import jax.experimental.pallas as pl
import jax.experimental.pallas.tpu as pltpu

F32 = jnp.float32
BF16 = jnp.bfloat16
U32 = jnp.uint32

LN_EPS = 1e-5
GRN_EPS = 1e-6
_C0 = 0.7978845608028654
_C1 = 0.044715
ALPHA = (_C0 * _C1) ** (1.0 / 3.0)
A0 = _C0 / ALPHA
KH = 0.5 / ALPHA


def _split_rows(total, parts, align=16):
    units = total // align
    base, rem = divmod(units, parts)
    sizes = [(base + (1 if k < rem else 0)) * align for k in range(parts)]
    offs = [sum(sizes[:k]) for k in range(parts)]
    return list(zip(offs, sizes))


def _kernel(x_hbm, dw_hbm, w1_hbm, w2_hbm, g_hbm, b_hbm,
            out_hbm, h_hbm,
            hpool, nbuf, xbuf, obuf, w1v, w2v, w2s, ssq, bias, dw_ref, g_ref, b_ref,
            hsem, xsem, osem, psem, wsem,
            *, T, S, tm, sub, nc, sub2, margin):
    C = x_hbm.shape[1]
    N = w1_hbm.shape[1]
    NH = T - S
    U = tm // sub
    U2 = tm // sub2

    def h_wr(tile, slot):
        return pltpu.make_async_copy(
            hpool.at[slot], h_hbm.at[pl.ds(tile * tm, tm), :], hsem.at[slot])

    def h_rd(tile, slot):
        return pltpu.make_async_copy(
            h_hbm.at[pl.ds(tile * tm, tm), :], hpool.at[slot], hsem.at[slot])

    def x_cp(tile, b):
        return pltpu.make_async_copy(
            x_hbm.at[pl.ds(tile * tm, tm), :], xbuf.at[b], xsem.at[b])

    def x0_cp(j):
        return pltpu.make_async_copy(
            x_hbm.at[pl.ds(j * sub, sub), :], xbuf.at[0, pl.ds(j * sub, sub), :], psem.at[j])

    def o_part(tile, b, j):
        return pltpu.make_async_copy(
            obuf.at[b, pl.ds(j * sub2, sub2), :],
            out_hbm.at[pl.ds(tile * tm + j * sub2, sub2), :], osem.at[b])

    def o_all(tile, b):
        return pltpu.make_async_copy(
            obuf.at[b], out_hbm.at[pl.ds(tile * tm, tm), :], osem.at[b])

    w1_cp = pltpu.make_async_copy(w1_hbm, w1v, wsem.at[0])
    w2_cp = pltpu.make_async_copy(w2_hbm, w2v, wsem.at[1])
    dw_cp = pltpu.make_async_copy(dw_hbm, dw_ref, wsem.at[2])
    g_cp = pltpu.make_async_copy(g_hbm, g_ref, wsem.at[3])
    b_cp = pltpu.make_async_copy(b_hbm, b_ref, wsem.at[4])

    def wrap(v, n):
        return jnp.where(v >= n, v - n, v)

    def ln_piece(xb, dst, r0, rows):
        dw = dw_ref[...].astype(F32)
        y = xbuf[xb, r0:r0 + rows, :].astype(F32) * dw
        m = jnp.sum(y, axis=-1, keepdims=True) * (1.0 / C)
        d = y - m
        ss = jnp.sum(d * d, axis=-1, keepdims=True)
        r = jnp.exp(jnp.log(ss + C * LN_EPS) * (-0.5) + math.log(ALPHA * C ** 0.5))
        n = (d * r).astype(BF16)
        nbuf[dst, r0 // 2:(r0 + rows) // 2, :] = pltpu.bitcast(n, U32)

    def mm1(cur, slot, j, c, order):
        r0 = j * sub
        parts = [pltpu.bitcast(nbuf[cur, (r0 + o) // 2:(r0 + o + r) // 2, :], BF16)
                 for (o, r) in order]
        lhs = parts[0] if len(parts) == 1 else jnp.concatenate(parts, axis=0)
        u = jnp.dot(lhs, w1v[:, c * nc:(c + 1) * nc], preferred_element_type=F32)
        h = u + u * jnp.tanh(u * (u * u + A0))
        pos = 0
        for (o, r) in order:
            hpool[slot, r0 + o:r0 + o + r, c * nc:(c + 1) * nc] = h[pos:pos + r, :].astype(BF16)
            pos += r
        ssq[:, c * nc:(c + 1) * nc] += (h * h).reshape(sub // 8, 8, nc).sum(axis=0)

    def x_seq(m):
        return jnp.where(m < T, m, wrap(m - T + NH, T))

    dw_cp.start()
    for j in range(U):
        x0_cp(j).start()
    w1_cp.start()
    x_cp(1, 1).start()
    w2_cp.start()
    g_cp.start()
    b_cp.start()
    ssq[...] = jnp.zeros_like(ssq)
    dw_cp.wait()
    for j in range(U):
        x0_cp(j).wait()
        for (o, r) in _split_rows(sub, max(sub // 256, 1)):
            ln_piece(0, 0, j * sub + o, r)
    x_cp(2, 0).start()
    w1_cp.wait()

    def phase0(i, slot):
        cur = i & 1
        nxt = 1 - cur
        x_cp(x_seq(i + 1), nxt).wait()

        @pl.when(i >= S)
        def _():
            h_wr(i - S, slot).wait()

        nch = N // nc
        sp = _split_rows(sub, nch)
        pieces = [(j * sub + o, r) for j in range(U) for (o, r) in sp]
        P = len(pieces)
        for j in range(U):
            for c in range(nch):
                order = [sp[k] for k in range(nch) if k != c] + [sp[c]]
                q = j * nch + c
                mm1(cur, slot, j, c, order)
                if q == P - 2:
                    ln_piece(nxt, nxt, *pieces[P - 1])
                    ln_piece(nxt, nxt, *pieces[0])
                elif q < P - 2:
                    ln_piece(nxt, nxt, *pieces[q + 1])

        @pl.when(i + 3 <= T + 1)
        def _():
            x_cp(x_seq(i + 3), nxt).start()

        @pl.when(i < NH)
        def _():
            h_wr(i, slot).start()

        return wrap(slot + 1, S)

    jax.lax.fori_loop(0, T, phase0, 0)

    w2_cp.wait()
    g_cp.wait()
    b_cp.wait()
    tot = jnp.sum(ssq[...], axis=0, keepdims=True) * (KH * KH)
    gx = jnp.sqrt(tot + GRN_EPS)
    nx = gx / (jnp.mean(gx, axis=-1, keepdims=True) + GRN_EPS)
    s = (1.0 + g_ref[...].astype(F32).reshape(1, N) * nx) * KH
    st = jnp.transpose(jnp.broadcast_to(s, (128, N)))
    w2 = w2v[...]
    w2f = w2.astype(F32)
    for c in range(C // 128):
        w2s[:, c * 128:(c + 1) * 128] = (w2f[:, c * 128:(c + 1) * 128] * st).astype(BF16)
    bias[...] = jnp.dot(jnp.broadcast_to(b_ref[...].astype(F32).reshape(1, N), (16, N)).astype(BF16), w2,
                        preferred_element_type=F32)[:8]

    num, den = (S - margin) + (NH - 1), (NH - 1)

    def phase1(i, carry):
        slot, tile, tile2, kk, kslot, acc = carry
        xb = (T + i) & 1
        ob = i & 1

        @pl.when(i >= 1)
        def _():
            x_cp(tile, xb).wait()

        @pl.when(i >= S)
        def _():
            h_rd(i - S, slot).wait()

        @pl.when(i >= 2)
        def _():
            o_all(tile2, ob).wait()

        bi = bias[0:1, :]
        for j in range(U2):
            r0 = j * sub2
            y = jnp.dot(hpool[slot, r0:r0 + sub2, :], w2s[...], preferred_element_type=F32)
            obuf[ob, r0:r0 + sub2, :] = (
                xbuf[xb, r0:r0 + sub2, :].astype(F32) + y + bi).astype(BF16)
            o_part(tile, ob, j).start()

        @pl.when(i + 2 < T)
        def _():
            x_cp(wrap(tile + 2, T), xb).start()

        hit = jnp.logical_and(acc < den, kk < NH)

        @pl.when(hit)
        def _():
            h_rd(kk, kslot).start(priority=1)

        acc = jnp.where(hit, acc + num, acc) - den
        kk = jnp.where(hit, kk + 1, kk)
        kslot = jnp.where(hit, wrap(kslot + 1, S), kslot)
        tile2 = wrap(tile + (T - 1), T)
        return wrap(slot + 1, S), wrap(tile + 1, T), tile2, kk, kslot, acc

    zero = jnp.int32(0)
    jax.lax.fori_loop(0, T, phase1,
                      (jnp.int32(NH % S), jnp.int32(NH % T), zero, zero, jnp.int32(NH % S), zero))
    o_all((NH + T - 2) % T, (T - 2) % 2).wait()
    o_all((NH + T - 1) % T, (T - 1) % 2).wait()


def _build(tm=3072, S=9, sub=512, nc=256, sub2=512, margin=3, vmem_mb=124):
    def fn(x, dw, w1, w2, grn_g, grn_b):
        B, H, W, C = x.shape
        M = B * H * W
        N = w1.shape[1]
        T = M // tm
        NH = T - S
        assert dw.shape[0] == 1 and dw.shape[1] == 1 and B == 1
        assert M % tm == 0 and NH >= 2 and T >= 3
        vm = pl.BlockSpec(memory_space=pltpu.VMEM)
        hbm = pl.BlockSpec(memory_space=pl.ANY)
        out, _ = pl.pallas_call(
            functools.partial(_kernel, T=T, S=S, tm=tm, sub=sub, nc=nc, sub2=sub2,
                              margin=margin),
            in_specs=[hbm] * 6,
            out_specs=[hbm, hbm],
            out_shape=[
                jax.ShapeDtypeStruct((M, C), BF16),
                jax.ShapeDtypeStruct((NH * tm, N), BF16),
            ],
            scratch_shapes=[
                pltpu.VMEM((S, tm, N), BF16),
                pltpu.VMEM((2, tm // 2, C), U32),
                pltpu.VMEM((2, tm, C), BF16),
                pltpu.VMEM((2, tm, C), BF16),
                pltpu.VMEM((C, N), BF16),
                pltpu.VMEM((N, C), BF16),
                pltpu.VMEM((N, C), BF16),
                pltpu.VMEM((8, N), F32),
                pltpu.VMEM((8, C), F32),
                pltpu.VMEM((1, C), BF16),
                pltpu.VMEM((N,), BF16),
                pltpu.VMEM((N,), BF16),
                pltpu.SemaphoreType.DMA((S,)),
                pltpu.SemaphoreType.DMA((2,)),
                pltpu.SemaphoreType.DMA((2,)),
                pltpu.SemaphoreType.DMA((tm // sub,)),
                pltpu.SemaphoreType.DMA((5,)),
            ],
            compiler_params=pltpu.CompilerParams(
                vmem_limit_bytes=vmem_mb * 1024 * 1024,
                disable_bounds_checks=True,
            ),
        )(x.reshape(M, C), dw.reshape(1, C), w1, w2, grn_g, grn_b)
        return out.reshape(B, H, W, C)

    return fn


_impl = _build()


@jax.jit
def pallas_standalone__modern_conv_block_slak__vision_kernel(
    x: jax.Array,
    dw: jax.Array,
    w1: jax.Array,
    w2: jax.Array,
    grn_g: jax.Array,
    grn_b: jax.Array,
):
    return _impl(x, dw, w1, w2, grn_g, grn_b)
```

```python
import functools
import math

import jax
import jax.numpy as jnp
import jax.experimental.pallas as pl
import jax.experimental.pallas.tpu as pltpu

F32 = jnp.float32
BF16 = jnp.bfloat16
U32 = jnp.uint32

LN_EPS = 1e-5
GRN_EPS = 1e-6
_C0 = 0.7978845608028654
_C1 = 0.044715
ALPHA = (_C0 * _C1) ** (1.0 / 3.0)
A0 = _C0 / ALPHA
KH = 0.5 / ALPHA
KSPLIT = 256


def _split_rows(total, parts, align=16):
    units = total // align
    base, rem = divmod(units, parts)
    sizes = [(base + (1 if k < rem else 0)) * align for k in range(parts)]
    offs = [sum(sizes[:k]) for k in range(parts)]
    return list(zip(offs, sizes))


def _kernel(x_hbm, dw_hbm, w1_hbm, w2_hbm, g_hbm, b_hbm,
            out_hbm, h_hbm,
            hpool, nbuf, xbuf, obuf, w1v, w2v, w2s, ssq, bias, dw_ref, g_ref, b_ref,
            hsem, xsem, osem, psem, wsem,
            *, T, S, tm, sub, nc, sub2, px, margin):
    C = x_hbm.shape[1]
    N = w1_hbm.shape[1]
    NH = T - S
    U = tm // sub
    U2 = tm // sub2

    def h_wr(tile, slot):
        return pltpu.make_async_copy(
            hpool.at[slot], h_hbm.at[pl.ds(tile * tm, tm), :], hsem.at[slot])

    def h_rd(tile, slot):
        return pltpu.make_async_copy(
            h_hbm.at[pl.ds(tile * tm, tm), :], hpool.at[slot], hsem.at[slot])

    def x_cp(tile, b):
        return pltpu.make_async_copy(
            x_hbm.at[pl.ds(tile * tm, tm), :], xbuf.at[b], xsem.at[b])

    def x0_cp(j):
        return pltpu.make_async_copy(
            x_hbm.at[pl.ds(j * px, px), :], xbuf.at[0, pl.ds(j * px, px), :], psem.at[j])

    def o_part(tile, b, j):
        return pltpu.make_async_copy(
            obuf.at[b, pl.ds(j * sub2, sub2), :],
            out_hbm.at[pl.ds(tile * tm + j * sub2, sub2), :], osem.at[b])

    def o_all(tile, b):
        return pltpu.make_async_copy(
            obuf.at[b], out_hbm.at[pl.ds(tile * tm, tm), :], osem.at[b])

    w1_cp = pltpu.make_async_copy(w1_hbm, w1v, wsem.at[0])
    w2_cp = pltpu.make_async_copy(w2_hbm, w2v, wsem.at[1])
    dw_cp = pltpu.make_async_copy(dw_hbm, dw_ref, wsem.at[2])
    g_cp = pltpu.make_async_copy(g_hbm, g_ref, wsem.at[3])
    b_cp = pltpu.make_async_copy(b_hbm, b_ref, wsem.at[4])

    def wrap(v, n):
        return jnp.where(v >= n, v - n, v)

    def ln_piece(xb, dst, r0, rows):
        dw = dw_ref[...].astype(F32)
        y = xbuf[xb, r0:r0 + rows, :].astype(F32) * dw
        m = jnp.sum(y, axis=-1, keepdims=True) * (1.0 / C)
        d = y - m
        ss = jnp.sum(d * d, axis=-1, keepdims=True)
        r = jnp.exp(jnp.log(ss + C * LN_EPS) * (-0.5) + math.log(ALPHA * C ** 0.5))
        n = (d * r).astype(BF16)
        nbuf[dst, r0 // 2:(r0 + rows) // 2, :] = pltpu.bitcast(n, U32)

    def mm1(cur, slot, j, c, order):
        r0 = j * sub
        parts = [pltpu.bitcast(nbuf[cur, (r0 + o) // 2:(r0 + o + r) // 2, :], BF16)
                 for (o, r) in order]
        lhs = parts[0] if len(parts) == 1 else jnp.concatenate(parts, axis=0)
        cols = slice(c * nc, (c + 1) * nc)
        u = (jnp.dot(lhs[:, :KSPLIT], w1v[:KSPLIT, cols], preferred_element_type=F32)
             + jnp.dot(lhs[:, KSPLIT:], w1v[KSPLIT:, cols], preferred_element_type=F32))
        h = u + u * jnp.tanh(u * (u * u + A0))
        pos = 0
        for (o, r) in order:
            hpool[slot, r0 + o:r0 + o + r, c * nc:(c + 1) * nc] = h[pos:pos + r, :].astype(BF16)
            pos += r
        ssq[:, c * nc:(c + 1) * nc] += (h * h).reshape(sub // 8, 8, nc).sum(axis=0)

    def x_seq(m):
        return jnp.where(m < T, m, wrap(m - T + NH, T))

    dw_cp.start()
    for j in range(tm // px):
        x0_cp(j).start()
    w1_cp.start()
    x_cp(1, 1).start()
    w2_cp.start()
    g_cp.start()
    b_cp.start()
    ssq[...] = jnp.zeros_like(ssq)
    dw_cp.wait()
    for j in range(tm // px):
        x0_cp(j).wait()
        for (o, r) in _split_rows(px, max(px // 256, 1)):
            ln_piece(0, 0, j * px + o, r)
    x_cp(2, 0).start()
    w1_cp.wait()

    def phase0(i, slot):
        cur = i & 1
        nxt = 1 - cur
        x_cp(x_seq(i + 1), nxt).wait()

        @pl.when(i >= S)
        def _():
            h_wr(i - S, slot).wait()

        nch = N // nc
        sp = _split_rows(sub, nch)
        for j in range(U):
            for c in range(nch):
                ln_piece(nxt, nxt, j * sub + sp[c][0], sp[c][1])
                mm1(cur, slot, j, c, [sp[k] for k in range(nch) if k != c] + [sp[c]])

        @pl.when(i + 3 <= T + 1)
        def _():
            x_cp(x_seq(i + 3), nxt).start()

        @pl.when(i < NH)
        def _():
            h_wr(i, slot).start()

        return wrap(slot + 1, S)

    jax.lax.fori_loop(0, T, phase0, 0)

    w2_cp.wait()
    g_cp.wait()
    b_cp.wait()
    tot = jnp.sum(ssq[...], axis=0, keepdims=True) * (KH * KH)
    gx = jnp.sqrt(tot + GRN_EPS)
    nx = gx / (jnp.mean(gx, axis=-1, keepdims=True) + GRN_EPS)
    s = (1.0 + g_ref[...].astype(F32).reshape(1, N) * nx) * KH
    st = jnp.transpose(jnp.broadcast_to(s, (128, N)))
    w2 = w2v[...]
    w2f = w2.astype(F32)
    for c in range(C // 128):
        w2s[:, c * 128:(c + 1) * 128] = (w2f[:, c * 128:(c + 1) * 128] * st).astype(BF16)
    bias[...] = jnp.dot(jnp.broadcast_to(b_ref[...].astype(F32).reshape(1, N), (16, N)).astype(BF16), w2,
                        preferred_element_type=F32)[:8]

    num, den = (S - margin) + (NH - 1), (NH - 1)

    def phase1(i, carry):
        slot, tile, tile2, kk, kslot, acc = carry
        xb = (T + i) & 1
        ob = i & 1

        @pl.when(i >= 1)
        def _():
            x_cp(tile, xb).wait()

        @pl.when(i >= S)
        def _():
            h_rd(i - S, slot).wait()

        @pl.when(i >= 2)
        def _():
            o_all(tile2, ob).wait()

        bi = bias[0:1, :]
        for j in range(U2):
            r0 = j * sub2
            y = jnp.dot(hpool[slot, r0:r0 + sub2, :], w2s[...], preferred_element_type=F32)
            obuf[ob, r0:r0 + sub2, :] = (
                xbuf[xb, r0:r0 + sub2, :].astype(F32) + y + bi).astype(BF16)
            o_part(tile, ob, j).start()

        @pl.when(i + 2 < T)
        def _():
            x_cp(wrap(tile + 2, T), xb).start()

        hit = jnp.logical_and(acc < den, kk < NH)

        @pl.when(hit)
        def _():
            h_rd(kk, kslot).start(priority=1)

        acc = jnp.where(hit, acc + num, acc) - den
        kk = jnp.where(hit, kk + 1, kk)
        kslot = jnp.where(hit, wrap(kslot + 1, S), kslot)
        tile2 = wrap(tile + (T - 1), T)
        return wrap(slot + 1, S), wrap(tile + 1, T), tile2, kk, kslot, acc

    zero = jnp.int32(0)
    jax.lax.fori_loop(0, T, phase1,
                      (jnp.int32(NH % S), jnp.int32(NH % T), zero, zero, jnp.int32(NH % S), zero))
    o_all((NH + T - 2) % T, (T - 2) % 2).wait()
    o_all((NH + T - 1) % T, (T - 1) % 2).wait()


def _build(tm=3072, S=9, sub=1024, nc=512, sub2=512, px=512, margin=3, vmem_mb=112):
    def fn(x, dw, w1, w2, grn_g, grn_b):
        B, H, W, C = x.shape
        M = B * H * W
        N = w1.shape[1]
        T = M // tm
        NH = T - S
        assert dw.shape[0] == 1 and dw.shape[1] == 1 and B == 1
        assert M % tm == 0 and NH >= 2 and T >= 3
        vm = pl.BlockSpec(memory_space=pltpu.VMEM)
        hbm = pl.BlockSpec(memory_space=pl.ANY)
        out, _ = pl.pallas_call(
            functools.partial(_kernel, T=T, S=S, tm=tm, sub=sub, nc=nc, sub2=sub2,
                              px=px, margin=margin),
            in_specs=[hbm] * 6,
            out_specs=[hbm, hbm],
            out_shape=[
                jax.ShapeDtypeStruct((M, C), BF16),
                jax.ShapeDtypeStruct((NH * tm, N), BF16),
            ],
            scratch_shapes=[
                pltpu.VMEM((S, tm, N), BF16),
                pltpu.VMEM((2, tm // 2, C), U32),
                pltpu.VMEM((2, tm, C), BF16),
                pltpu.VMEM((2, tm, C), BF16),
                pltpu.VMEM((C, N), BF16),
                pltpu.VMEM((N, C), BF16),
                pltpu.VMEM((N, C), BF16),
                pltpu.VMEM((8, N), F32),
                pltpu.VMEM((8, C), F32),
                pltpu.VMEM((1, C), BF16),
                pltpu.VMEM((N,), BF16),
                pltpu.VMEM((N,), BF16),
                pltpu.SemaphoreType.DMA((S,)),
                pltpu.SemaphoreType.DMA((2,)),
                pltpu.SemaphoreType.DMA((2,)),
                pltpu.SemaphoreType.DMA((tm // px,)),
                pltpu.SemaphoreType.DMA((5,)),
            ],
            compiler_params=pltpu.CompilerParams(
                vmem_limit_bytes=vmem_mb * 1024 * 1024,
                disable_bounds_checks=True,
            ),
        )(x.reshape(M, C), dw.reshape(1, C), w1, w2, grn_g, grn_b)
        return out.reshape(B, H, W, C)

    return fn


_impl = _build()


@jax.jit
def pallas_standalone__modern_conv_block_slak__vision_kernel(
    x: jax.Array,
    dw: jax.Array,
    w1: jax.Array,
    w2: jax.Array,
    grn_g: jax.Array,
    grn_b: jax.Array,
):
    return _impl(x, dw, w1, w2, grn_g, grn_b)
```

```python
import functools
import math

import jax
import jax.numpy as jnp
import jax.experimental.pallas as pl
import jax.experimental.pallas.tpu as pltpu

F32 = jnp.float32
BF16 = jnp.bfloat16
U32 = jnp.uint32

LN_EPS = 1e-5
GRN_EPS = 1e-6
_C0 = 0.7978845608028654
_C1 = 0.044715
ALPHA = (_C0 * _C1) ** (1.0 / 3.0)
A0 = _C0 / ALPHA
KH = 0.5 / ALPHA
KSPLIT = 256


def _split_rows(total, parts, align=16):
    units = total // align
    base, rem = divmod(units, parts)
    sizes = [(base + (1 if k < rem else 0)) * align for k in range(parts)]
    offs = [sum(sizes[:k]) for k in range(parts)]
    return list(zip(offs, sizes))


def _kernel(x_hbm, dw_hbm, w1_hbm, w2_hbm, g_hbm, b_hbm,
            out_hbm, h_hbm,
            hpool, nbuf, xbuf, obuf, w1v, w2v, w2s, ssq, bias, dw_ref, g_ref, b_ref,
            hsem, xsem, osem, psem, wsem,
            *, T, S, tm, sub, nc, sub2, px, margin):
    C = x_hbm.shape[1]
    N = w1_hbm.shape[1]
    NH = T - S
    U = tm // sub
    U2 = tm // sub2

    def h_wr(tile, slot):
        return pltpu.make_async_copy(
            hpool.at[slot], h_hbm.at[pl.ds(tile * tm, tm), :], hsem.at[slot])

    def h_rd(tile, slot):
        return pltpu.make_async_copy(
            h_hbm.at[pl.ds(tile * tm, tm), :], hpool.at[slot], hsem.at[slot])

    def xa_cp(tile, b):
        return pltpu.make_async_copy(
            x_hbm.at[pl.ds(tile * tm, sub), :], xbuf.at[b, pl.ds(0, sub), :], xsem.at[b])

    def xb_cp(tile, b):
        return pltpu.make_async_copy(
            x_hbm.at[pl.ds(tile * tm + sub, tm - sub), :], xbuf.at[b, pl.ds(sub, tm - sub), :],
            xsem.at[3 + b])

    def x0_cp(j):
        return pltpu.make_async_copy(
            x_hbm.at[pl.ds(j * px, px), :], xbuf.at[0, pl.ds(j * px, px), :], psem.at[j])

    def o_part(tile, b, j):
        return pltpu.make_async_copy(
            obuf.at[b, pl.ds(j * sub2, sub2), :],
            out_hbm.at[pl.ds(tile * tm + j * sub2, sub2), :], osem.at[b])

    def o_all(tile, b):
        return pltpu.make_async_copy(
            obuf.at[b], out_hbm.at[pl.ds(tile * tm, tm), :], osem.at[b])

    w1_cp = pltpu.make_async_copy(w1_hbm, w1v, wsem.at[0])
    w2_cp = pltpu.make_async_copy(w2_hbm, w2v, wsem.at[1])
    dw_cp = pltpu.make_async_copy(dw_hbm, dw_ref, wsem.at[2])
    g_cp = pltpu.make_async_copy(g_hbm, g_ref, wsem.at[3])
    b_cp = pltpu.make_async_copy(b_hbm, b_ref, wsem.at[4])

    def wrap(v, n):
        return jnp.where(v >= n, v - n, v)

    def ln_piece(xb, src0, dst, r0, rows):
        dw = dw_ref[...].astype(F32)
        y = xbuf[xb, src0:src0 + rows, :].astype(F32) * dw
        m = jnp.sum(y, axis=-1, keepdims=True) * (1.0 / C)
        d = y - m
        ss = jnp.sum(d * d, axis=-1, keepdims=True)
        r = jnp.exp(jnp.log(ss + C * LN_EPS) * (-0.5) + math.log(ALPHA * C ** 0.5))
        n = (d * r).astype(BF16)
        nbuf[dst, r0 // 2:(r0 + rows) // 2, :] = pltpu.bitcast(n, U32)

    def mm1(cur, slot, j, c, order):
        r0 = j * sub
        parts = [pltpu.bitcast(nbuf[cur, o // 2:(o + r) // 2, :], BF16) for (o, r) in order]
        lhs = parts[0] if len(parts) == 1 else jnp.concatenate(parts, axis=0)
        cols = slice(c * nc, (c + 1) * nc)
        u = (jnp.dot(lhs[:, :KSPLIT], w1v[:KSPLIT, cols], preferred_element_type=F32)
             + jnp.dot(lhs[:, KSPLIT:], w1v[KSPLIT:, cols], preferred_element_type=F32))
        h = u + u * jnp.tanh(u * (u * u + A0))
        pos = 0
        for (o, r) in order:
            hpool[slot, r0 + o:r0 + o + r, c * nc:(c + 1) * nc] = h[pos:pos + r, :].astype(BF16)
            pos += r
        ssq[:, c * nc:(c + 1) * nc] += (h * h).reshape(sub // 8, 8, nc).sum(axis=0)

    def x_seq(m):
        return jnp.where(m < T, m, wrap(m - T + NH, T))

    def x_top(m, b, bn):
        xb_cp(x_seq(m), b).wait()

        @pl.when(m + 1 < 2 * T)
        def _():
            xa_cp(x_seq(m + 1), bn).wait()

    def x_bottom(m, b):
        @pl.when(m + 3 < 2 * T)
        def _():
            t = x_seq(m + 3)
            xa_cp(t, b).start()
            xb_cp(t, b).start()

    dw_cp.start()
    for j in range(sub // px):
        x0_cp(j).start()
    w1_cp.start()
    xb_cp(0, 0).start()
    xa_cp(1, 1).start()
    ssq[...] = jnp.zeros_like(ssq)
    dw_cp.wait()
    for j in range(sub // px):
        x0_cp(j).wait()
        for (o, r) in _split_rows(px, max(px // 256, 1)):
            ln_piece(0, j * px + o, 0, j * px + o, r)
    w1_cp.wait()
    xb_cp(1, 1).start()
    xa_cp(2, 2).start()
    xb_cp(2, 2).start()
    w2_cp.start()
    g_cp.start()
    b_cp.start()

    def phase0(i, carry):
        slot, b = carry
        bn = wrap(b + 1, 3)
        x_top(i, b, bn)

        @pl.when(i >= S)
        def _():
            h_wr(i - S, slot).wait()

        nch = N // nc
        sp = _split_rows(sub, nch)
        for j in range(U):
            cur = (i * U + j) & 1
            nxt = 1 - cur
            for c in range(nch):
                if j + 1 < U:
                    ln_piece(b, (j + 1) * sub + sp[c][0], nxt, sp[c][0], sp[c][1])
                else:
                    ln_piece(bn, sp[c][0], nxt, sp[c][0], sp[c][1])
                mm1(cur, slot, j, c, [sp[k] for k in range(nch) if k != c] + [sp[c]])

        x_bottom(i, b)

        @pl.when(i < NH)
        def _():
            h_wr(i, slot).start()

        return wrap(slot + 1, S), bn

    jax.lax.fori_loop(0, T, phase0, (jnp.int32(0), jnp.int32(0)))

    w2_cp.wait()
    g_cp.wait()
    b_cp.wait()
    tot = jnp.sum(ssq[...], axis=0, keepdims=True) * (KH * KH)
    gx = jnp.sqrt(tot + GRN_EPS)
    nx = gx / (jnp.mean(gx, axis=-1, keepdims=True) + GRN_EPS)
    s = (1.0 + g_ref[...].astype(F32).reshape(1, N) * nx) * KH
    st = jnp.transpose(jnp.broadcast_to(s, (128, N)))
    w2 = w2v[...]
    w2f = w2.astype(F32)
    for c in range(C // 128):
        w2s[:, c * 128:(c + 1) * 128] = (w2f[:, c * 128:(c + 1) * 128] * st).astype(BF16)
    bias[...] = jnp.dot(jnp.broadcast_to(b_ref[...].astype(F32).reshape(1, N), (16, N)).astype(BF16), w2,
                        preferred_element_type=F32)[:8]

    num, den = (S - margin) + (NH - 1), (NH - 1)

    def phase1(i, carry):
        slot, tile, tile2, kk, kslot, acc, xb = carry
        ob = i & 1
        x_top(T + i, xb, wrap(xb + 1, 3))

        @pl.when(i >= S)
        def _():
            h_rd(i - S, slot).wait()

        @pl.when(i >= 2)
        def _():
            o_all(tile2, ob).wait()

        bi = bias[0:1, :]
        for j in range(U2):
            r0 = j * sub2
            y = jnp.dot(hpool[slot, r0:r0 + sub2, :], w2s[...], preferred_element_type=F32)
            obuf[ob, r0:r0 + sub2, :] = (
                xbuf[xb, r0:r0 + sub2, :].astype(F32) + y + bi).astype(BF16)
            o_part(tile, ob, j).start()

        x_bottom(T + i, xb)

        hit = jnp.logical_and(acc < den, kk < NH)

        @pl.when(hit)
        def _():
            h_rd(kk, kslot).start(priority=1)

        acc = jnp.where(hit, acc + num, acc) - den
        kk = jnp.where(hit, kk + 1, kk)
        kslot = jnp.where(hit, wrap(kslot + 1, S), kslot)
        tile2 = wrap(tile + (T - 1), T)
        return (wrap(slot + 1, S), wrap(tile + 1, T), tile2, kk, kslot, acc, wrap(xb + 1, 3))

    zero = jnp.int32(0)
    jax.lax.fori_loop(0, T, phase1,
                      (jnp.int32(NH % S), jnp.int32(NH % T), zero, zero, jnp.int32(NH % S), zero,
                       jnp.int32(T % 3)))
    o_all((NH + T - 2) % T, (T - 2) % 2).wait()
    o_all((NH + T - 1) % T, (T - 1) % 2).wait()


def _build(tm=3072, S=9, sub=1024, nc=512, sub2=512, px=512, margin=3, vmem_mb=112):
    def fn(x, dw, w1, w2, grn_g, grn_b):
        B, H, W, C = x.shape
        M = B * H * W
        N = w1.shape[1]
        T = M // tm
        NH = T - S
        assert dw.shape[0] == 1 and dw.shape[1] == 1 and B == 1
        assert M % tm == 0 and NH >= 2 and T >= 3
        vm = pl.BlockSpec(memory_space=pltpu.VMEM)
        hbm = pl.BlockSpec(memory_space=pl.ANY)
        out, _ = pl.pallas_call(
            functools.partial(_kernel, T=T, S=S, tm=tm, sub=sub, nc=nc, sub2=sub2,
                              px=px, margin=margin),
            in_specs=[hbm] * 6,
            out_specs=[hbm, hbm],
            out_shape=[
                jax.ShapeDtypeStruct((M, C), BF16),
                jax.ShapeDtypeStruct((NH * tm, N), BF16),
            ],
            scratch_shapes=[
                pltpu.VMEM((S, tm, N), BF16),
                pltpu.VMEM((2, sub // 2, C), U32),
                pltpu.VMEM((3, tm, C), BF16),
                pltpu.VMEM((2, tm, C), BF16),
                pltpu.VMEM((C, N), BF16),
                pltpu.VMEM((N, C), BF16),
                pltpu.VMEM((N, C), BF16),
                pltpu.VMEM((8, N), F32),
                pltpu.VMEM((8, C), F32),
                pltpu.VMEM((1, C), BF16),
                pltpu.VMEM((N,), BF16),
                pltpu.VMEM((N,), BF16),
                pltpu.SemaphoreType.DMA((S,)),
                pltpu.SemaphoreType.DMA((6,)),
                pltpu.SemaphoreType.DMA((2,)),
                pltpu.SemaphoreType.DMA((sub // px,)),
                pltpu.SemaphoreType.DMA((5,)),
            ],
            compiler_params=pltpu.CompilerParams(
                vmem_limit_bytes=vmem_mb * 1024 * 1024,
                disable_bounds_checks=True,
            ),
        )(x.reshape(M, C), dw.reshape(1, C), w1, w2, grn_g, grn_b)
        return out.reshape(B, H, W, C)

    return fn


_impl = _build()


@jax.jit
def pallas_standalone__modern_conv_block_slak__vision_kernel(
    x: jax.Array,
    dw: jax.Array,
    w1: jax.Array,
    w2: jax.Array,
    grn_g: jax.Array,
    grn_b: jax.Array,
):
    return _impl(x, dw, w1, w2, grn_g, grn_b)
```

```python
import functools
import math

import jax
import jax.numpy as jnp
import jax.experimental.pallas as pl
import jax.experimental.pallas.tpu as pltpu

F32 = jnp.float32
BF16 = jnp.bfloat16
U32 = jnp.uint32

LN_EPS = 1e-5
GRN_EPS = 1e-6
_C0 = 0.7978845608028654
_C1 = 0.044715
ALPHA = (_C0 * _C1) ** (1.0 / 3.0)
A0 = _C0 / ALPHA
KH = 0.5 / ALPHA
KSPLIT = 256


def _split_rows(total, parts, align=16):
    units = total // align
    base, rem = divmod(units, parts)
    sizes = [(base + (1 if k < rem else 0)) * align for k in range(parts)]
    offs = [sum(sizes[:k]) for k in range(parts)]
    return list(zip(offs, sizes))


def _kernel(x_hbm, dw_hbm, w1_hbm, w2_hbm, g_hbm, b_hbm,
            out_hbm, h_hbm,
            hpool, nbuf, xbuf, obuf, w1v, w2v, w2s, ssq, bias, dw_ref, g_ref, b_ref,
            hsem, xsem, osem, psem, wsem,
            *, T, S, tm, sub, nc, sub2, px, margin, ppc):
    C = x_hbm.shape[1]
    N = w1_hbm.shape[1]
    NH = T - S
    U = tm // sub
    U2 = tm // sub2

    def h_wr(tile, slot):
        return pltpu.make_async_copy(
            hpool.at[slot], h_hbm.at[pl.ds(tile * tm, tm), :], hsem.at[slot])

    def h_rd(tile, slot):
        return pltpu.make_async_copy(
            h_hbm.at[pl.ds(tile * tm, tm), :], hpool.at[slot], hsem.at[slot])

    def xa_cp(tile, b):
        return pltpu.make_async_copy(
            x_hbm.at[pl.ds(tile * tm, sub), :], xbuf.at[b, pl.ds(0, sub), :], xsem.at[b])

    def xb_cp(tile, b):
        return pltpu.make_async_copy(
            x_hbm.at[pl.ds(tile * tm + sub, tm - sub), :], xbuf.at[b, pl.ds(sub, tm - sub), :],
            xsem.at[3 + b])

    def x0_cp(j):
        return pltpu.make_async_copy(
            x_hbm.at[pl.ds(j * px, px), :], xbuf.at[0, pl.ds(j * px, px), :], psem.at[j])

    def o_part(tile, b, j):
        return pltpu.make_async_copy(
            obuf.at[b, pl.ds(j * sub2, sub2), :],
            out_hbm.at[pl.ds(tile * tm + j * sub2, sub2), :], osem.at[b])

    def o_all(tile, b):
        return pltpu.make_async_copy(
            obuf.at[b], out_hbm.at[pl.ds(tile * tm, tm), :], osem.at[b])

    w1_cp = pltpu.make_async_copy(w1_hbm, w1v, wsem.at[0])
    w2_cp = pltpu.make_async_copy(w2_hbm, w2v, wsem.at[1])
    dw_cp = pltpu.make_async_copy(dw_hbm, dw_ref, wsem.at[2])
    g_cp = pltpu.make_async_copy(g_hbm, g_ref, wsem.at[3])
    b_cp = pltpu.make_async_copy(b_hbm, b_ref, wsem.at[4])

    def wrap(v, n):
        return jnp.where(v >= n, v - n, v)

    def ln_piece(xb, src0, dst, r0, rows):
        dw = dw_ref[...].astype(F32)
        y = xbuf[xb, src0:src0 + rows, :].astype(F32) * dw
        m = jnp.sum(y, axis=-1, keepdims=True) * (1.0 / C)
        d = y - m
        ss = jnp.sum(d * d, axis=-1, keepdims=True)
        r = jnp.exp(jnp.log(ss + C * LN_EPS) * (-0.5) + math.log(ALPHA * C ** 0.5))
        n = (d * r).astype(BF16)
        nbuf[dst, r0 // 2:(r0 + rows) // 2, :] = pltpu.bitcast(n, U32)

    def mm1(cur, slot, j, c, order):
        r0 = j * sub
        parts = [pltpu.bitcast(nbuf[cur, o // 2:(o + r) // 2, :], BF16) for (o, r) in order]
        lhs = parts[0] if len(parts) == 1 else jnp.concatenate(parts, axis=0)
        cols = slice(c * nc, (c + 1) * nc)
        u = (jnp.dot(lhs[:, :KSPLIT], w1v[:KSPLIT, cols], preferred_element_type=F32)
             + jnp.dot(lhs[:, KSPLIT:], w1v[KSPLIT:, cols], preferred_element_type=F32))
        h = u + u * jnp.tanh(u * (u * u + A0))
        pos = 0
        for (o, r) in order:
            hpool[slot, r0 + o:r0 + o + r, c * nc:(c + 1) * nc] = h[pos:pos + r, :].astype(BF16)
            pos += r
        ssq[:, c * nc:(c + 1) * nc] += (h * h).reshape(sub // 8, 8, nc).sum(axis=0)

    def x_seq(m):
        return jnp.where(m < T, m, wrap(m - T + NH, T))

    def x_top(m, b, bn):
        xb_cp(x_seq(m), b).wait()

        @pl.when(m + 1 < 2 * T)
        def _():
            xa_cp(x_seq(m + 1), bn).wait()

    def x_bottom(m, b):
        @pl.when(m + 3 < 2 * T)
        def _():
            t = x_seq(m + 3)
            xa_cp(t, b).start()
            xb_cp(t, b).start()

    dw_cp.start()
    for j in range(sub // px):
        x0_cp(j).start()
    w1_cp.start()
    xb_cp(0, 0).start()
    xa_cp(1, 1).start()
    ssq[...] = jnp.zeros_like(ssq)
    dw_cp.wait()
    for j in range(sub // px):
        x0_cp(j).wait()
        for (o, r) in _split_rows(px, max(px // 256, 1)):
            ln_piece(0, j * px + o, 0, j * px + o, r)
    w1_cp.wait()
    xb_cp(1, 1).start()
    xa_cp(2, 2).start()
    xb_cp(2, 2).start()
    w2_cp.start()
    g_cp.start()
    b_cp.start()

    def phase0(i, carry):
        slot, b = carry
        bn = wrap(b + 1, 3)
        x_top(i, b, bn)

        @pl.when(i >= S)
        def _():
            h_wr(i - S, slot).wait()

        nch = N // nc
        npc = nch * ppc
        sp = _split_rows(sub, npc)
        for j in range(U):
            cur = (i * U + j) & 1
            nxt = 1 - cur
            for c in range(nch):
                pinned = list(range(c * ppc, (c + 1) * ppc))
                for k in pinned:
                    if j + 1 < U:
                        ln_piece(b, (j + 1) * sub + sp[k][0], nxt, sp[k][0], sp[k][1])
                    else:
                        ln_piece(bn, sp[k][0], nxt, sp[k][0], sp[k][1])
                order = [sp[k] for k in range(npc) if k not in pinned] + [sp[k] for k in pinned]
                mm1(cur, slot, j, c, order)

        x_bottom(i, b)

        @pl.when(i < NH)
        def _():
            h_wr(i, slot).start()

        return wrap(slot + 1, S), bn

    jax.lax.fori_loop(0, T, phase0, (jnp.int32(0), jnp.int32(0)))

    w2_cp.wait()
    g_cp.wait()
    b_cp.wait()
    tot = jnp.sum(ssq[...], axis=0, keepdims=True) * (KH * KH)
    gx = jnp.sqrt(tot + GRN_EPS)
    nx = gx / (jnp.mean(gx, axis=-1, keepdims=True) + GRN_EPS)
    s = (1.0 + g_ref[...].astype(F32).reshape(1, N) * nx) * KH
    st = jnp.transpose(jnp.broadcast_to(s, (128, N)))
    w2 = w2v[...]
    w2f = w2.astype(F32)
    for c in range(C // 128):
        w2s[:, c * 128:(c + 1) * 128] = (w2f[:, c * 128:(c + 1) * 128] * st).astype(BF16)
    brow = jnp.broadcast_to(b_ref[...].astype(F32).reshape(1, N), (16, N)).astype(BF16)
    bias[...] = jnp.dot(brow, w2, preferred_element_type=F32)[:8]

    num, den = (S - margin) + (NH - 1), (NH - 1)

    def phase1(i, carry):
        slot, tile, tile2, kk, kslot, acc, xb = carry
        ob = i & 1
        x_top(T + i, xb, wrap(xb + 1, 3))

        @pl.when(i >= S)
        def _():
            h_rd(i - S, slot).wait()

        @pl.when(i >= 2)
        def _():
            o_all(tile2, ob).wait()

        bi = bias[0:1, :]
        for j in range(U2):
            r0 = j * sub2
            y = jnp.dot(hpool[slot, r0:r0 + sub2, :], w2s[...], preferred_element_type=F32)
            obuf[ob, r0:r0 + sub2, :] = (
                xbuf[xb, r0:r0 + sub2, :].astype(F32) + y + bi).astype(BF16)
            o_part(tile, ob, j).start()

        x_bottom(T + i, xb)

        hit = jnp.logical_and(acc < den, kk < NH)

        @pl.when(hit)
        def _():
            h_rd(kk, kslot).start(priority=1)

        acc = jnp.where(hit, acc + num, acc) - den
        kk = jnp.where(hit, kk + 1, kk)
        kslot = jnp.where(hit, wrap(kslot + 1, S), kslot)
        tile2 = wrap(tile + (T - 1), T)
        return (wrap(slot + 1, S), wrap(tile + 1, T), tile2, kk, kslot, acc, wrap(xb + 1, 3))

    zero = jnp.int32(0)
    jax.lax.fori_loop(0, T, phase1,
                      (jnp.int32(NH % S), jnp.int32(NH % T), zero, zero, jnp.int32(NH % S), zero,
                       jnp.int32(T % 3)))
    o_all((NH + T - 2) % T, (T - 2) % 2).wait()
    o_all((NH + T - 1) % T, (T - 1) % 2).wait()


def _build(tm=3072, S=9, sub=768, nc=512, sub2=512, px=256, margin=3, vmem_mb=112, ppc=4):
    def fn(x, dw, w1, w2, grn_g, grn_b):
        B, H, W, C = x.shape
        M = B * H * W
        N = w1.shape[1]
        T = M // tm
        NH = T - S
        assert dw.shape[0] == 1 and dw.shape[1] == 1 and B == 1
        assert M % tm == 0 and NH >= 2 and T >= 3
        hbm = pl.BlockSpec(memory_space=pl.ANY)
        out, _ = pl.pallas_call(
            functools.partial(_kernel, T=T, S=S, tm=tm, sub=sub, nc=nc, sub2=sub2,
                              px=px, margin=margin, ppc=ppc),
            in_specs=[hbm] * 6,
            out_specs=[hbm, hbm],
            out_shape=[
                jax.ShapeDtypeStruct((M, C), BF16),
                jax.ShapeDtypeStruct((NH * tm, N), BF16),
            ],
            scratch_shapes=[
                pltpu.VMEM((S, tm, N), BF16),
                pltpu.VMEM((2, sub // 2, C), U32),
                pltpu.VMEM((3, tm, C), BF16),
                pltpu.VMEM((2, tm, C), BF16),
                pltpu.VMEM((C, N), BF16),
                pltpu.VMEM((N, C), BF16),
                pltpu.VMEM((N, C), BF16),
                pltpu.VMEM((8, N), F32),
                pltpu.VMEM((8, C), F32),
                pltpu.VMEM((1, C), BF16),
                pltpu.VMEM((N,), BF16),
                pltpu.VMEM((N,), BF16),
                pltpu.SemaphoreType.DMA((S,)),
                pltpu.SemaphoreType.DMA((6,)),
                pltpu.SemaphoreType.DMA((2,)),
                pltpu.SemaphoreType.DMA((sub // px,)),
                pltpu.SemaphoreType.DMA((5,)),
            ],
            compiler_params=pltpu.CompilerParams(
                vmem_limit_bytes=vmem_mb * 1024 * 1024,
                disable_bounds_checks=True,
            ),
        )(x.reshape(M, C), dw.reshape(1, C), w1, w2, grn_g, grn_b)
        return out.reshape(B, H, W, C)

    return fn


_impl = _build()


@jax.jit
def pallas_standalone__modern_conv_block_slak__vision_kernel(
    x: jax.Array,
    dw: jax.Array,
    w1: jax.Array,
    w2: jax.Array,
    grn_g: jax.Array,
    grn_b: jax.Array,
):
    return _impl(x, dw, w1, w2, grn_g, grn_b)
```

```python
import functools
import math

import jax
import jax.numpy as jnp
import jax.experimental.pallas as pl
import jax.experimental.pallas.tpu as pltpu

F32 = jnp.float32
BF16 = jnp.bfloat16
U32 = jnp.uint32

LN_EPS = 1e-5
GRN_EPS = 1e-6
_C0 = 0.7978845608028654
_C1 = 0.044715
ALPHA = (_C0 * _C1) ** (1.0 / 3.0)
A0 = _C0 / ALPHA
KH = 0.5 / ALPHA
KSPLIT = 256


def _split_rows(total, parts, align=16):
    units = total // align
    base, rem = divmod(units, parts)
    sizes = [(base + (1 if k < rem else 0)) * align for k in range(parts)]
    offs = [sum(sizes[:k]) for k in range(parts)]
    return list(zip(offs, sizes))


def _kernel(x_hbm, dw_hbm, w1_hbm, w2_hbm, g_hbm, b_hbm,
            out_hbm, h_hbm,
            hpool, nbuf, xbuf, obuf, w1v, w2v, w2s, ssq, bias, dw_ref, g_ref, b_ref,
            hsem, xsem, osem, psem, wsem,
            *, T, S, tm, sub, nc, sub2, px, margin, ppc):
    C = x_hbm.shape[1]
    N = w1_hbm.shape[1]
    NH = T - S
    U = tm // sub
    U2 = tm // sub2

    def h_wr(tile, slot):
        return pltpu.make_async_copy(
            hpool.at[slot], h_hbm.at[pl.ds(tile * tm, tm), :], hsem.at[slot])

    def h_rd(tile, slot):
        return pltpu.make_async_copy(
            h_hbm.at[pl.ds(tile * tm, tm), :], hpool.at[slot], hsem.at[slot])

    def xa_cp(tile, b):
        return pltpu.make_async_copy(
            x_hbm.at[pl.ds(tile * tm, sub), :], xbuf.at[b, pl.ds(0, sub), :], xsem.at[b])

    def xb_cp(tile, b):
        return pltpu.make_async_copy(
            x_hbm.at[pl.ds(tile * tm + sub, tm - sub), :], xbuf.at[b, pl.ds(sub, tm - sub), :],
            xsem.at[3 + b])

    NPX = sub // px

    def x0_cp(k):
        return pltpu.make_async_copy(
            x_hbm.at[pl.ds(k * px, px), :], xbuf.at[0, pl.ds(k * px, px), :], psem.at[k])

    def x0_part(j):
        return pltpu.make_async_copy(
            x_hbm.at[pl.ds(j * sub, sub), :], xbuf.at[0, pl.ds(j * sub, sub), :],
            psem.at[NPX + j - 1])

    def o_part(tile, b, j):
        return pltpu.make_async_copy(
            obuf.at[b, pl.ds(j * sub2, sub2), :],
            out_hbm.at[pl.ds(tile * tm + j * sub2, sub2), :], osem.at[b])

    def o_all(tile, b):
        return pltpu.make_async_copy(
            obuf.at[b], out_hbm.at[pl.ds(tile * tm, tm), :], osem.at[b])

    w1_cp = pltpu.make_async_copy(w1_hbm, w1v, wsem.at[0])
    w2_cp = pltpu.make_async_copy(w2_hbm, w2v, wsem.at[1])
    dw_cp = pltpu.make_async_copy(dw_hbm, dw_ref, wsem.at[2])
    g_cp = pltpu.make_async_copy(g_hbm, g_ref, wsem.at[3])
    b_cp = pltpu.make_async_copy(b_hbm, b_ref, wsem.at[4])

    def wrap(v, n):
        return jnp.where(v >= n, v - n, v)

    def ln_piece(xb, src0, dst, r0, rows):
        dw = dw_ref[...].astype(F32)
        y = xbuf[xb, pl.ds(src0, rows), :].astype(F32) * dw
        m = jnp.sum(y, axis=-1, keepdims=True) * (1.0 / C)
        d = y - m
        ss = jnp.sum(d * d, axis=-1, keepdims=True)
        r = jnp.exp(jnp.log(ss + C * LN_EPS) * (-0.5) + math.log(ALPHA * C ** 0.5))
        n = (d * r).astype(BF16)
        nbuf[dst, r0 // 2:(r0 + rows) // 2, :] = pltpu.bitcast(n, U32)

    def mm1(cur, slot, r0, c, order):
        parts = [pltpu.bitcast(nbuf[cur, o // 2:(o + r) // 2, :], BF16) for (o, r) in order]
        lhs = parts[0] if len(parts) == 1 else jnp.concatenate(parts, axis=0)
        cols = slice(c * nc, (c + 1) * nc)
        u = (jnp.dot(lhs[:, :KSPLIT], w1v[:KSPLIT, cols], preferred_element_type=F32)
             + jnp.dot(lhs[:, KSPLIT:], w1v[KSPLIT:, cols], preferred_element_type=F32))
        h = u + u * jnp.tanh(u * (u * u + A0))
        pos = 0
        for (o, r) in order:
            hpool[slot, pl.ds(r0 + o, r), cols] = h[pos:pos + r, :].astype(BF16)
            pos += r
        ssq[:, cols] += (h * h).reshape(sub // 8, 8, nc).sum(axis=0)

    def sub_tile(slot, r0, cur, xsrc, xrow):
        nxt = 1 - cur
        nch = N // nc
        npc = nch * ppc
        sp = _split_rows(sub, npc)
        for c in range(nch):
            pinned = list(range(c * ppc, (c + 1) * ppc))
            for k in pinned:
                ln_piece(xsrc, xrow + sp[k][0], nxt, sp[k][0], sp[k][1])
            order = [sp[k] for k in range(npc) if k not in pinned] + [sp[k] for k in pinned]
            mm1(cur, slot, r0, c, order)

    def x_seq(m):
        return jnp.where(m < T, m, wrap(m - T + NH, T))

    def x_top(m, b, bn):
        xb_cp(x_seq(m), b).wait()

        @pl.when(m + 1 < 2 * T)
        def _():
            xa_cp(x_seq(m + 1), bn).wait()

    def x_bottom(m, b):
        @pl.when(m + 3 < 2 * T)
        def _():
            t = x_seq(m + 3)
            xa_cp(t, b).start()
            xb_cp(t, b).start()

    dw_cp.start()
    for k in range(NPX):
        x0_cp(k).start()
    w1_cp.start()
    x0_part(1).start()
    ssq[...] = jnp.zeros_like(ssq)
    dw_cp.wait()
    for k in range(NPX):
        x0_cp(k).wait()
        for (o, r) in _split_rows(px, max(px // 256, 1)):
            ln_piece(0, k * px + o, 0, k * px + o, r)
    w1_cp.wait()
    for j in range(2, U):
        x0_part(j).start()
    xa_cp(1, 1).start()
    xb_cp(1, 1).start()
    xa_cp(2, 2).start()
    xb_cp(2, 2).start()
    w2_cp.start()
    g_cp.start()
    b_cp.start()

    def tile0(j, carry):
        inner = j + 1 < U

        @pl.when(inner)
        def _():
            x0_part(j + 1).wait()

        @pl.when(jnp.logical_not(inner))
        def _():
            xa_cp(1, 1).wait()

        sub_tile(0, pl.multiple_of(j * sub, sub), j & 1, jnp.where(inner, 0, 1),
                 pl.multiple_of(jnp.where(inner, (j + 1) * sub, 0), sub))
        return carry

    jax.lax.fori_loop(0, U, tile0, 0)
    x_bottom(0, 0)
    h_wr(0, 0).start()

    def phase0(i, carry):
        slot, b = carry
        bn = wrap(b + 1, 3)
        x_top(i, b, bn)

        @pl.when(i >= S)
        def _():
            h_wr(i - S, slot).wait()

        for j in range(U):
            cur = (i * U + j) & 1
            if j + 1 < U:
                sub_tile(slot, j * sub, cur, b, (j + 1) * sub)
            else:
                sub_tile(slot, j * sub, cur, bn, 0)

        x_bottom(i, b)

        @pl.when(i < NH)
        def _():
            h_wr(i, slot).start()

        return wrap(slot + 1, S), bn

    jax.lax.fori_loop(1, T, phase0, (jnp.int32(1 % S), jnp.int32(1)))

    w2_cp.wait()
    g_cp.wait()
    b_cp.wait()
    tot = jnp.sum(ssq[...], axis=0, keepdims=True) * (KH * KH)
    gx = jnp.sqrt(tot + GRN_EPS)
    nx = gx / (jnp.mean(gx, axis=-1, keepdims=True) + GRN_EPS)
    s = (1.0 + g_ref[...].astype(F32).reshape(1, N) * nx) * KH
    st = jnp.transpose(jnp.broadcast_to(s, (128, N)))
    w2 = w2v[...]
    w2f = w2.astype(F32)
    for c in range(C // 128):
        w2s[:, c * 128:(c + 1) * 128] = (w2f[:, c * 128:(c + 1) * 128] * st).astype(BF16)
    brow = jnp.broadcast_to(b_ref[...].astype(F32).reshape(1, N), (16, N)).astype(BF16)
    bias[...] = jnp.dot(brow, w2, preferred_element_type=F32)[:8]

    num, den = (S - margin) + (NH - 1), (NH - 1)

    def phase1(i, carry):
        slot, tile, tile2, kk, kslot, acc, xb = carry
        ob = i & 1
        x_top(T + i, xb, wrap(xb + 1, 3))

        @pl.when(i >= S)
        def _():
            h_rd(i - S, slot).wait()

        @pl.when(i >= 2)
        def _():
            o_all(tile2, ob).wait()

        bi = bias[0:1, :]
        for j in range(U2):
            r0 = j * sub2
            y = jnp.dot(hpool[slot, r0:r0 + sub2, :], w2s[...], preferred_element_type=F32)
            obuf[ob, r0:r0 + sub2, :] = (
                xbuf[xb, r0:r0 + sub2, :].astype(F32) + y + bi).astype(BF16)
            o_part(tile, ob, j).start()

        x_bottom(T + i, xb)

        hit = jnp.logical_and(acc < den, kk < NH)

        @pl.when(hit)
        def _():
            h_rd(kk, kslot).start(priority=1)

        acc = jnp.where(hit, acc + num, acc) - den
        kk = jnp.where(hit, kk + 1, kk)
        kslot = jnp.where(hit, wrap(kslot + 1, S), kslot)
        tile2 = wrap(tile + (T - 1), T)
        return (wrap(slot + 1, S), wrap(tile + 1, T), tile2, kk, kslot, acc, wrap(xb + 1, 3))

    zero = jnp.int32(0)
    jax.lax.fori_loop(0, T, phase1,
                      (jnp.int32(NH % S), jnp.int32(NH % T), zero, zero, jnp.int32(NH % S), zero,
                       jnp.int32(T % 3)))
    o_all((NH + T - 2) % T, (T - 2) % 2).wait()
    o_all((NH + T - 1) % T, (T - 1) % 2).wait()


def _build(tm=3072, S=9, sub=768, nc=512, sub2=512, px=256, margin=3, vmem_mb=112, ppc=4):
    def fn(x, dw, w1, w2, grn_g, grn_b):
        B, H, W, C = x.shape
        M = B * H * W
        N = w1.shape[1]
        T = M // tm
        NH = T - S
        assert dw.shape[0] == 1 and dw.shape[1] == 1 and B == 1
        assert M % tm == 0 and NH >= 2 and T >= 3
        hbm = pl.BlockSpec(memory_space=pl.ANY)
        out, _ = pl.pallas_call(
            functools.partial(_kernel, T=T, S=S, tm=tm, sub=sub, nc=nc, sub2=sub2,
                              px=px, margin=margin, ppc=ppc),
            in_specs=[hbm] * 6,
            out_specs=[hbm, hbm],
            out_shape=[
                jax.ShapeDtypeStruct((M, C), BF16),
                jax.ShapeDtypeStruct((NH * tm, N), BF16),
            ],
            scratch_shapes=[
                pltpu.VMEM((S, tm, N), BF16),
                pltpu.VMEM((2, sub // 2, C), U32),
                pltpu.VMEM((3, tm, C), BF16),
                pltpu.VMEM((2, tm, C), BF16),
                pltpu.VMEM((C, N), BF16),
                pltpu.VMEM((N, C), BF16),
                pltpu.VMEM((N, C), BF16),
                pltpu.VMEM((8, N), F32),
                pltpu.VMEM((8, C), F32),
                pltpu.VMEM((1, C), BF16),
                pltpu.VMEM((N,), BF16),
                pltpu.VMEM((N,), BF16),
                pltpu.SemaphoreType.DMA((S,)),
                pltpu.SemaphoreType.DMA((6,)),
                pltpu.SemaphoreType.DMA((2,)),
                pltpu.SemaphoreType.DMA((sub // px + tm // sub - 1,)),
                pltpu.SemaphoreType.DMA((5,)),
            ],
            compiler_params=pltpu.CompilerParams(
                vmem_limit_bytes=vmem_mb * 1024 * 1024,
                disable_bounds_checks=True,
            ),
        )(x.reshape(M, C), dw.reshape(1, C), w1, w2, grn_g, grn_b)
        return out.reshape(B, H, W, C)

    return fn


_impl = _build()


@jax.jit
def pallas_standalone__modern_conv_block_slak__vision_kernel(
    x: jax.Array,
    dw: jax.Array,
    w1: jax.Array,
    w2: jax.Array,
    grn_g: jax.Array,
    grn_b: jax.Array,
):
    return _impl(x, dw, w1, w2, grn_g, grn_b)
```

```python
import functools
import math

import jax
import jax.numpy as jnp
import jax.experimental.pallas as pl
import jax.experimental.pallas.tpu as pltpu

F32 = jnp.float32
BF16 = jnp.bfloat16
U32 = jnp.uint32

LN_EPS = 1e-5
GRN_EPS = 1e-6
_C0 = 0.7978845608028654
_C1 = 0.044715
ALPHA = (_C0 * _C1) ** (1.0 / 3.0)
A0 = _C0 / ALPHA
KH = 0.5 / ALPHA
KSPLIT = 256


def _split_rows(total, parts, align=16):
    units = total // align
    base, rem = divmod(units, parts)
    sizes = [(base + (1 if k < rem else 0)) * align for k in range(parts)]
    offs = [sum(sizes[:k]) for k in range(parts)]
    return list(zip(offs, sizes))


def _kernel(x_hbm, dw_hbm, w1_hbm, w2_hbm, g_hbm, b_hbm,
            out_hbm, h_hbm,
            hpool, nbuf, xbuf, obuf, w1v, w2v, w2s, ssq, bias, dw_ref, g_ref, b_ref,
            hsem, xsem, osem, psem, wsem,
            *, T, S, tm, sub, nc, sub2, px, margin, ppc):
    C = x_hbm.shape[1]
    N = w1_hbm.shape[1]
    NH = T - S
    U = tm // sub
    U2 = tm // sub2

    def h_wr(tile, slot):
        return pltpu.make_async_copy(
            hpool.at[slot], h_hbm.at[pl.ds(tile * tm, tm), :], hsem.at[slot])

    def h_rd(tile, slot):
        return pltpu.make_async_copy(
            h_hbm.at[pl.ds(tile * tm, tm), :], hpool.at[slot], hsem.at[slot])

    def xa_cp(tile, b):
        return pltpu.make_async_copy(
            x_hbm.at[pl.ds(tile * tm, sub), :], xbuf.at[b, pl.ds(0, sub), :], xsem.at[b])

    def xb_cp(tile, b):
        return pltpu.make_async_copy(
            x_hbm.at[pl.ds(tile * tm + sub, tm - sub), :], xbuf.at[b, pl.ds(sub, tm - sub), :],
            xsem.at[3 + b])

    NPX = sub // px

    def x0_cp(k):
        return pltpu.make_async_copy(
            x_hbm.at[pl.ds(k * px, px), :], xbuf.at[0, pl.ds(k * px, px), :], psem.at[k])

    def x0_part(j):
        return pltpu.make_async_copy(
            x_hbm.at[pl.ds(j * sub, sub), :], xbuf.at[0, pl.ds(j * sub, sub), :],
            psem.at[NPX + j - 1])

    def o_part(tile, b, j):
        return pltpu.make_async_copy(
            obuf.at[b, pl.ds(j * sub2, sub2), :],
            out_hbm.at[pl.ds(tile * tm + j * sub2, sub2), :], osem.at[b])

    def o_all(tile, b):
        return pltpu.make_async_copy(
            obuf.at[b], out_hbm.at[pl.ds(tile * tm, tm), :], osem.at[b])

    def w1_cp(c):
        return pltpu.make_async_copy(
            w1_hbm.at[:, pl.ds(c * nc, nc)], w1v.at[:, pl.ds(c * nc, nc)], wsem.at[4 + c])

    w2_cp = pltpu.make_async_copy(w2_hbm, w2v, wsem.at[0])
    dw_cp = pltpu.make_async_copy(dw_hbm, dw_ref, wsem.at[1])
    g_cp = pltpu.make_async_copy(g_hbm, g_ref, wsem.at[2])
    b_cp = pltpu.make_async_copy(b_hbm, b_ref, wsem.at[3])

    def wrap(v, n):
        return jnp.where(v >= n, v - n, v)

    def ln_piece(xb, src0, dst, r0, rows):
        dw = dw_ref[...].astype(F32)
        y = xbuf[xb, pl.ds(src0, rows), :].astype(F32) * dw
        m = jnp.sum(y, axis=-1, keepdims=True) * (1.0 / C)
        d = y - m
        ss = jnp.sum(d * d, axis=-1, keepdims=True)
        r = jnp.exp(jnp.log(ss + C * LN_EPS) * (-0.5) + math.log(ALPHA * C ** 0.5))
        n = (d * r).astype(BF16)
        nbuf[dst, r0 // 2:(r0 + rows) // 2, :] = pltpu.bitcast(n, U32)

    def mm1(cur, slot, r0, c, order):
        parts = [pltpu.bitcast(nbuf[cur, o // 2:(o + r) // 2, :], BF16) for (o, r) in order]
        lhs = parts[0] if len(parts) == 1 else jnp.concatenate(parts, axis=0)
        cols = slice(c * nc, (c + 1) * nc)
        u = (jnp.dot(lhs[:, :KSPLIT], w1v[:KSPLIT, cols], preferred_element_type=F32)
             + jnp.dot(lhs[:, KSPLIT:], w1v[KSPLIT:, cols], preferred_element_type=F32))
        h = u + u * jnp.tanh(u * (u * u + A0))
        pos = 0
        for (o, r) in order:
            hpool[slot, pl.ds(r0 + o, r), cols] = h[pos:pos + r, :].astype(BF16)
            pos += r
        ssq[:, cols] += (h * h).reshape(sub // 8, 8, nc).sum(axis=0)

    def sub_tile(slot, r0, cur, xsrc, xrow, first=False):
        nxt = 1 - cur
        nch = N // nc
        npc = nch * ppc
        sp = _split_rows(sub, npc)
        for c in range(nch):
            if first:
                w1_cp(c).wait()
                if c == 1:
                    x0_part(1).wait()
                half = npc // 2
                pinned = [[], list(range(half)), list(range(half, npc))][c] if c < 3 else []
            else:
                pinned = list(range(c * ppc, (c + 1) * ppc))
            for k in pinned:
                ln_piece(xsrc, xrow + sp[k][0], nxt, sp[k][0], sp[k][1])
            order = [sp[k] for k in range(npc) if k not in pinned] + [sp[k] for k in pinned]
            mm1(cur, slot, r0, c, order)

    def x_seq(m):
        return jnp.where(m < T, m, wrap(m - T + NH, T))

    def x_top(m, b, bn):
        xb_cp(x_seq(m), b).wait()

        @pl.when(m + 1 < 2 * T)
        def _():
            xa_cp(x_seq(m + 1), bn).wait()

    def x_bottom(m, b):
        @pl.when(m + 3 < 2 * T)
        def _():
            t = x_seq(m + 3)
            xa_cp(t, b).start()
            xb_cp(t, b).start()

    dw_cp.start()
    for k in range(NPX):
        x0_cp(k).start()
    w1_cp(0).start()
    x0_part(1).start()
    ssq[...] = jnp.zeros_like(ssq)
    dw_cp.wait()
    for k in range(NPX):
        x0_cp(k).wait()
        if k == 0:
            for c in range(1, N // nc):
                w1_cp(c).start()
        for (o, r) in _split_rows(px, max(px // 256, 1)):
            ln_piece(0, k * px + o, 0, k * px + o, r)
    for j in range(2, U):
        x0_part(j).start()
    xa_cp(1, 1).start()
    sub_tile(0, 0, 0, 0, sub, first=True)
    xb_cp(1, 1).start()
    xa_cp(2, 2).start()
    xb_cp(2, 2).start()
    w2_cp.start()
    g_cp.start()
    b_cp.start()

    def tile0(j, carry):
        inner = j + 1 < U

        @pl.when(inner)
        def _():
            x0_part(j + 1).wait()

        @pl.when(jnp.logical_not(inner))
        def _():
            xa_cp(1, 1).wait()

        sub_tile(0, pl.multiple_of(j * sub, sub), j & 1, jnp.where(inner, 0, 1),
                 pl.multiple_of(jnp.where(inner, (j + 1) * sub, 0), sub))
        return carry

    jax.lax.fori_loop(1, U, tile0, 0)
    x_bottom(0, 0)
    h_wr(0, 0).start()

    def phase0(i, carry):
        slot, b = carry
        bn = wrap(b + 1, 3)
        x_top(i, b, bn)

        @pl.when(i >= S)
        def _():
            h_wr(i - S, slot).wait()

        for j in range(U):
            cur = (i * U + j) & 1
            if j + 1 < U:
                sub_tile(slot, j * sub, cur, b, (j + 1) * sub)
            else:
                sub_tile(slot, j * sub, cur, bn, 0)

        x_bottom(i, b)

        @pl.when(i < NH)
        def _():
            h_wr(i, slot).start()

        return wrap(slot + 1, S), bn

    jax.lax.fori_loop(1, T, phase0, (jnp.int32(1 % S), jnp.int32(1)))

    w2_cp.wait()
    g_cp.wait()
    b_cp.wait()
    tot = jnp.sum(ssq[...], axis=0, keepdims=True) * (KH * KH)
    gx = jnp.sqrt(tot + GRN_EPS)
    nx = gx / (jnp.mean(gx, axis=-1, keepdims=True) + GRN_EPS)
    s = (1.0 + g_ref[...].astype(F32).reshape(1, N) * nx) * KH
    st = jnp.transpose(jnp.broadcast_to(s, (128, N)))
    w2 = w2v[...]
    w2f = w2.astype(F32)
    for c in range(C // 128):
        w2s[:, c * 128:(c + 1) * 128] = (w2f[:, c * 128:(c + 1) * 128] * st).astype(BF16)
    brow = jnp.broadcast_to(b_ref[...].astype(F32).reshape(1, N), (16, N)).astype(BF16)
    bias[...] = jnp.dot(brow, w2, preferred_element_type=F32)[:8]

    num, den = (S - margin) + (NH - 1), (NH - 1)

    def phase1(i, carry):
        slot, tile, tile2, kk, kslot, acc, xb = carry
        ob = i & 1
        x_top(T + i, xb, wrap(xb + 1, 3))

        @pl.when(i >= S)
        def _():
            h_rd(i - S, slot).wait()

        @pl.when(i >= 2)
        def _():
            o_all(tile2, ob).wait()

        bi = bias[0:1, :]
        for j in range(U2):
            r0 = j * sub2
            y = jnp.dot(hpool[slot, r0:r0 + sub2, :], w2s[...], preferred_element_type=F32)
            obuf[ob, r0:r0 + sub2, :] = (
                xbuf[xb, r0:r0 + sub2, :].astype(F32) + y + bi).astype(BF16)
            o_part(tile, ob, j).start()

        x_bottom(T + i, xb)

        hit = jnp.logical_and(acc < den, kk < NH)

        @pl.when(hit)
        def _():
            h_rd(kk, kslot).start(priority=1)

        acc = jnp.where(hit, acc + num, acc) - den
        kk = jnp.where(hit, kk + 1, kk)
        kslot = jnp.where(hit, wrap(kslot + 1, S), kslot)
        tile2 = wrap(tile + (T - 1), T)
        return (wrap(slot + 1, S), wrap(tile + 1, T), tile2, kk, kslot, acc, wrap(xb + 1, 3))

    zero = jnp.int32(0)
    jax.lax.fori_loop(0, T, phase1,
                      (jnp.int32(NH % S), jnp.int32(NH % T), zero, zero, jnp.int32(NH % S), zero,
                       jnp.int32(T % 3)))
    o_all((NH + T - 2) % T, (T - 2) % 2).wait()
    o_all((NH + T - 1) % T, (T - 1) % 2).wait()


def _build(tm=3072, S=9, sub=768, nc=512, sub2=512, px=256, margin=3, vmem_mb=112, ppc=4):
    def fn(x, dw, w1, w2, grn_g, grn_b):
        B, H, W, C = x.shape
        M = B * H * W
        N = w1.shape[1]
        T = M // tm
        NH = T - S
        assert dw.shape[0] == 1 and dw.shape[1] == 1 and B == 1
        assert M % tm == 0 and NH >= 2 and S >= 2 and tm // sub >= 2 and N // nc >= 3
        hbm = pl.BlockSpec(memory_space=pl.ANY)
        out, _ = pl.pallas_call(
            functools.partial(_kernel, T=T, S=S, tm=tm, sub=sub, nc=nc, sub2=sub2,
                              px=px, margin=margin, ppc=ppc),
            in_specs=[hbm] * 6,
            out_specs=[hbm, hbm],
            out_shape=[
                jax.ShapeDtypeStruct((M, C), BF16),
                jax.ShapeDtypeStruct((NH * tm, N), BF16),
            ],
            scratch_shapes=[
                pltpu.VMEM((S, tm, N), BF16),
                pltpu.VMEM((2, sub // 2, C), U32),
                pltpu.VMEM((3, tm, C), BF16),
                pltpu.VMEM((2, tm, C), BF16),
                pltpu.VMEM((C, N), BF16),
                pltpu.VMEM((N, C), BF16),
                pltpu.VMEM((N, C), BF16),
                pltpu.VMEM((8, N), F32),
                pltpu.VMEM((8, C), F32),
                pltpu.VMEM((1, C), BF16),
                pltpu.VMEM((N,), BF16),
                pltpu.VMEM((N,), BF16),
                pltpu.SemaphoreType.DMA((S,)),
                pltpu.SemaphoreType.DMA((6,)),
                pltpu.SemaphoreType.DMA((2,)),
                pltpu.SemaphoreType.DMA((sub // px + tm // sub - 1,)),
                pltpu.SemaphoreType.DMA((4 + N // nc,)),
            ],
            compiler_params=pltpu.CompilerParams(
                vmem_limit_bytes=vmem_mb * 1024 * 1024,
                disable_bounds_checks=True,
            ),
        )(x.reshape(M, C), dw.reshape(1, C), w1, w2, grn_g, grn_b)
        return out.reshape(B, H, W, C)

    return fn


_impl = _build()


@jax.jit
def pallas_standalone__modern_conv_block_slak__vision_kernel(
    x: jax.Array,
    dw: jax.Array,
    w1: jax.Array,
    w2: jax.Array,
    grn_g: jax.Array,
    grn_b: jax.Array,
):
    return _impl(x, dw, w1, w2, grn_g, grn_b)
```

```python
import functools
import math

import jax
import jax.numpy as jnp
import jax.experimental.pallas as pl
import jax.experimental.pallas.tpu as pltpu

F32 = jnp.float32
BF16 = jnp.bfloat16
U32 = jnp.uint32

LN_EPS = 1e-5
GRN_EPS = 1e-6
_C0 = 0.7978845608028654
_C1 = 0.044715
ALPHA = (_C0 * _C1) ** (1.0 / 3.0)
A0 = _C0 / ALPHA
KH = 0.5 / ALPHA
KSPLIT = 256


def _split_rows(total, parts, align=16):
    units = total // align
    base, rem = divmod(units, parts)
    sizes = [(base + (1 if k < rem else 0)) * align for k in range(parts)]
    offs = [sum(sizes[:k]) for k in range(parts)]
    return list(zip(offs, sizes))


def _kernel(x_hbm, dw_hbm, w1_hbm, w2_hbm, g_hbm, b_hbm,
            out_hbm, h_hbm,
            hpool, nbuf, xbuf, obuf, w1v, w2v, w2s, ssq, bias, dw_ref, g_ref, b_ref,
            hsem, xsem, osem, psem, wsem,
            *, T, S, tm, sub, nc, sub2, px, margin, ppc):
    C = x_hbm.shape[1]
    N = w1_hbm.shape[1]
    NH = T - S
    U = tm // sub
    U2 = tm // sub2

    def h_wr(tile, slot):
        return pltpu.make_async_copy(
            hpool.at[slot], h_hbm.at[pl.ds(tile * tm, tm), :], hsem.at[slot])

    def h_rd(tile, slot):
        return pltpu.make_async_copy(
            h_hbm.at[pl.ds(tile * tm, tm), :], hpool.at[slot], hsem.at[slot])

    def xa_cp(tile, b):
        return pltpu.make_async_copy(
            x_hbm.at[pl.ds(tile * tm, sub), :], xbuf.at[b, pl.ds(0, sub), :], xsem.at[b])

    def xb_cp(tile, b):
        return pltpu.make_async_copy(
            x_hbm.at[pl.ds(tile * tm + sub, tm - sub), :], xbuf.at[b, pl.ds(sub, tm - sub), :],
            xsem.at[3 + b])

    NPX = sub // px

    def x0_cp(k):
        return pltpu.make_async_copy(
            x_hbm.at[pl.ds(k * px, px), :], xbuf.at[0, pl.ds(k * px, px), :], psem.at[k])

    def x0_part(j):
        return pltpu.make_async_copy(
            x_hbm.at[pl.ds(j * sub, sub), :], xbuf.at[0, pl.ds(j * sub, sub), :],
            psem.at[NPX + j - 1])

    def o_part(tile, b, j):
        return pltpu.make_async_copy(
            obuf.at[b, pl.ds(j * sub2, sub2), :],
            out_hbm.at[pl.ds(tile * tm + j * sub2, sub2), :], osem.at[b])

    def o_all(tile, b):
        return pltpu.make_async_copy(
            obuf.at[b], out_hbm.at[pl.ds(tile * tm, tm), :], osem.at[b])

    def w1_cp(c):
        return pltpu.make_async_copy(
            w1_hbm.at[:, pl.ds(c * nc, nc)], w1v.at[:, pl.ds(c * nc, nc)], wsem.at[4 + c])

    w2_cp = pltpu.make_async_copy(w2_hbm, w2v, wsem.at[0])
    dw_cp = pltpu.make_async_copy(dw_hbm, dw_ref, wsem.at[1])
    g_cp = pltpu.make_async_copy(g_hbm, g_ref, wsem.at[2])
    b_cp = pltpu.make_async_copy(b_hbm, b_ref, wsem.at[3])

    def wrap(v, n):
        return jnp.where(v >= n, v - n, v)

    def ln_piece(xb, src0, dst, r0, rows):
        dw = dw_ref[...].astype(F32)
        y = xbuf[xb, pl.ds(src0, rows), :].astype(F32) * dw
        m = jnp.sum(y, axis=-1, keepdims=True) * (1.0 / C)
        d = y - m
        ss = jnp.sum(d * d, axis=-1, keepdims=True)
        r = jnp.exp(jnp.log(ss + C * LN_EPS) * (-0.5) + math.log(ALPHA * C ** 0.5))
        n = (d * r).astype(BF16)
        nbuf[dst, r0 // 2:(r0 + rows) // 2, :] = pltpu.bitcast(n, U32)

    def mm1(cur, slot, r0, c, order):
        parts = [pltpu.bitcast(nbuf[cur, o // 2:(o + r) // 2, :], BF16) for (o, r) in order]
        lhs = parts[0] if len(parts) == 1 else jnp.concatenate(parts, axis=0)
        cols = slice(c * nc, (c + 1) * nc)
        u = (jnp.dot(lhs[:, :KSPLIT], w1v[:KSPLIT, cols], preferred_element_type=F32)
             + jnp.dot(lhs[:, KSPLIT:], w1v[KSPLIT:, cols], preferred_element_type=F32))
        h = u + u * jnp.tanh(u * (u * u + A0))
        pos = 0
        for (o, r) in order:
            hpool[slot, pl.ds(r0 + o, r), cols] = h[pos:pos + r, :].astype(BF16)
            pos += r
        ssq[:, cols] += (h * h).reshape(sub // 8, 8, nc).sum(axis=0)

    def sub_tile(slot, r0, cur, xsrc, xrow, first=False):
        nxt = 1 - cur
        nch = N // nc
        npc = nch * ppc
        sp = _split_rows(sub, npc)
        for c in range(nch):
            if first:
                w1_cp(c).wait()
                if c == 1:
                    x0_part(1).wait()
                half = npc // 2
                pinned = [[], list(range(half)), list(range(half, npc))][c] if c < 3 else []
            else:
                pinned = list(range(c * ppc, (c + 1) * ppc))
            for k in pinned:
                ln_piece(xsrc, xrow + sp[k][0], nxt, sp[k][0], sp[k][1])
            order = [sp[k] for k in range(npc) if k not in pinned] + [sp[k] for k in pinned]
            mm1(cur, slot, r0, c, order)

    def x_seq(m):
        return jnp.minimum(jnp.where(m < T, m, wrap(m - T + NH, T)), T - 1)

    def x_top(m, b, bn):
        xb_cp(x_seq(m), b).wait()

        @pl.when(m + 1 < 2 * T)
        def _():
            xa_cp(x_seq(m + 1), bn).wait()

    def x_bottom(m, b):
        @pl.when(m + 3 < 2 * T)
        def _():
            t = x_seq(m + 3)
            xa_cp(t, b).start()
            xb_cp(t, b).start()

    dw_cp.start()
    for k in range(NPX):
        x0_cp(k).start()
    w1_cp(0).start()
    x0_part(1).start()
    ssq[...] = jnp.zeros_like(ssq)
    dw_cp.wait()
    for k in range(NPX):
        x0_cp(k).wait()
        if k == 0:
            for c in range(1, N // nc):
                w1_cp(c).start()
        for (o, r) in _split_rows(px, max(px // 256, 1)):
            ln_piece(0, k * px + o, 0, k * px + o, r)
    for j in range(2, U):
        x0_part(j).start()
    xa_cp(1, 1).start()
    sub_tile(0, 0, 0, 0, sub, first=True)
    xb_cp(1, 1).start()
    xa_cp(2, 2).start()
    xb_cp(2, 2).start()
    w2_cp.start()
    g_cp.start()
    b_cp.start()

    def tile0(j, carry):
        inner = j + 1 < U

        @pl.when(inner)
        def _():
            x0_part(jnp.minimum(j + 1, U - 1)).wait()

        @pl.when(jnp.logical_not(inner))
        def _():
            xa_cp(1, 1).wait()

        sub_tile(0, pl.multiple_of(j * sub, sub), j & 1, jnp.where(inner, 0, 1),
                 pl.multiple_of(jnp.where(inner, (j + 1) * sub, 0), sub))
        return carry

    jax.lax.fori_loop(1, U, tile0, 0)
    x_bottom(0, 0)
    h_wr(0, 0).start()

    def phase0(i, carry):
        slot, b = carry
        bn = wrap(b + 1, 3)
        x_top(i, b, bn)

        @pl.when(i >= S)
        def _():
            h_wr(jnp.maximum(i - S, 0), slot).wait()

        for j in range(U):
            cur = (i * U + j) & 1
            if j + 1 < U:
                sub_tile(slot, j * sub, cur, b, (j + 1) * sub)
            else:
                sub_tile(slot, j * sub, cur, bn, 0)

        x_bottom(i, b)

        @pl.when(i < NH)
        def _():
            h_wr(jnp.minimum(i, NH - 1), slot).start()

        return wrap(slot + 1, S), bn

    jax.lax.fori_loop(1, T, phase0, (jnp.int32(1 % S), jnp.int32(1)))

    w2_cp.wait()
    g_cp.wait()
    b_cp.wait()
    tot = jnp.sum(ssq[...], axis=0, keepdims=True) * (KH * KH)
    gx = jnp.sqrt(tot + GRN_EPS)
    nx = gx / (jnp.mean(gx, axis=-1, keepdims=True) + GRN_EPS)
    s = (1.0 + g_ref[...].astype(F32).reshape(1, N) * nx) * KH
    st = jnp.transpose(jnp.broadcast_to(s, (128, N)))
    w2 = w2v[...]
    w2f = w2.astype(F32)
    for c in range(C // 128):
        w2s[:, c * 128:(c + 1) * 128] = (w2f[:, c * 128:(c + 1) * 128] * st).astype(BF16)
    brow = jnp.broadcast_to(b_ref[...].astype(F32).reshape(1, N), (16, N)).astype(BF16)
    bias[...] = jnp.dot(brow, w2, preferred_element_type=F32)[:8]

    num, den = (S - margin) + (NH - 1), (NH - 1)

    def phase1(i, carry):
        slot, tile, tile2, kk, kslot, acc, xb = carry
        ob = i & 1
        x_top(T + i, xb, wrap(xb + 1, 3))

        @pl.when(i >= S)
        def _():
            h_rd(jnp.maximum(i - S, 0), slot).wait()

        @pl.when(i >= 2)
        def _():
            o_all(tile2, ob).wait()

        bi = bias[0:1, :]
        for j in range(U2):
            r0 = j * sub2
            y = jnp.dot(hpool[slot, r0:r0 + sub2, :], w2s[...], preferred_element_type=F32)
            obuf[ob, r0:r0 + sub2, :] = (
                xbuf[xb, r0:r0 + sub2, :].astype(F32) + y + bi).astype(BF16)
            o_part(tile, ob, j).start()

        x_bottom(T + i, xb)

        hit = jnp.logical_and(acc < den, kk < NH)

        @pl.when(hit)
        def _():
            h_rd(jnp.minimum(kk, NH - 1), kslot).start(priority=1)

        acc = jnp.where(hit, acc + num, acc) - den
        kk = jnp.where(hit, kk + 1, kk)
        kslot = jnp.where(hit, wrap(kslot + 1, S), kslot)
        tile2 = wrap(tile + (T - 1), T)
        return (wrap(slot + 1, S), wrap(tile + 1, T), tile2, kk, kslot, acc, wrap(xb + 1, 3))

    zero = jnp.int32(0)
    jax.lax.fori_loop(0, T, phase1,
                      (jnp.int32(NH % S), jnp.int32(NH % T), zero, zero, jnp.int32(NH % S), zero,
                       jnp.int32(T % 3)))
    o_all((NH + T - 2) % T, (T - 2) % 2).wait()
    o_all((NH + T - 1) % T, (T - 1) % 2).wait()


def _build(tm=3072, S=9, sub=768, nc=512, sub2=512, px=256, margin=3, vmem_mb=112, ppc=4):
    def fn(x, dw, w1, w2, grn_g, grn_b):
        B, H, W, C = x.shape
        M = B * H * W
        N = w1.shape[1]
        T = M // tm
        NH = T - S
        assert dw.shape[0] == 1 and dw.shape[1] == 1 and B == 1
        assert M % tm == 0 and NH >= 2 and S >= 2 and tm // sub >= 2 and N // nc >= 3
        hbm = pl.BlockSpec(memory_space=pl.ANY)
        out, _ = pl.pallas_call(
            functools.partial(_kernel, T=T, S=S, tm=tm, sub=sub, nc=nc, sub2=sub2,
                              px=px, margin=margin, ppc=ppc),
            in_specs=[hbm] * 6,
            out_specs=[hbm, hbm],
            out_shape=[
                jax.ShapeDtypeStruct((M, C), BF16),
                jax.ShapeDtypeStruct((NH * tm, N), BF16),
            ],
            scratch_shapes=[
                pltpu.VMEM((S, tm, N), BF16),
                pltpu.VMEM((2, sub // 2, C), U32),
                pltpu.VMEM((3, tm, C), BF16),
                pltpu.VMEM((2, tm, C), BF16),
                pltpu.VMEM((C, N), BF16),
                pltpu.VMEM((N, C), BF16),
                pltpu.VMEM((N, C), BF16),
                pltpu.VMEM((8, N), F32),
                pltpu.VMEM((8, C), F32),
                pltpu.VMEM((1, C), BF16),
                pltpu.VMEM((N,), BF16),
                pltpu.VMEM((N,), BF16),
                pltpu.SemaphoreType.DMA((S,)),
                pltpu.SemaphoreType.DMA((6,)),
                pltpu.SemaphoreType.DMA((2,)),
                pltpu.SemaphoreType.DMA((sub // px + tm // sub - 1,)),
                pltpu.SemaphoreType.DMA((4 + N // nc,)),
            ],
            compiler_params=pltpu.CompilerParams(
                vmem_limit_bytes=vmem_mb * 1024 * 1024,
                disable_bounds_checks=True,
            ),
        )(x.reshape(M, C), dw.reshape(1, C), w1, w2, grn_g, grn_b)
        return out.reshape(B, H, W, C)

    return fn


_impl = _build()


@jax.jit
def pallas_standalone__modern_conv_block_slak__vision_kernel(
    x: jax.Array,
    dw: jax.Array,
    w1: jax.Array,
    w2: jax.Array,
    grn_g: jax.Array,
    grn_b: jax.Array,
):
    return _impl(x, dw, w1, w2, grn_g, grn_b)
```
